```python
import jax
import jax.numpy as jnp

def _softmax(x, axis=-1):
    return jax.nn.softmax(x, axis=axis)
def _gelu(x):
    return jax.nn.gelu(x, approximate=True)
def _silu(x):
    return jax.nn.silu(x)
def _sigmoid(x):
    return jax.nn.sigmoid(x)
def _layernorm(x, axis=-1, eps=1e-5):
    m = jnp.mean(x, axis=axis, keepdims=True)
    v = jnp.var(x, axis=axis, keepdims=True)
    return (x - m) / jnp.sqrt(v + eps)
def _scatter_add(tgt, idx, src, axis=0):
    return tgt.at[idx].add(src)
def _segment_sum(src, seg, n):
    return jax.ops.segment_sum(src, seg, n)
class _Rng:
    def __init__(self, key):
        self._k = key
    def _next(self):
        self._k, sub = jax.random.split(self._k)
        return sub
    def normal(self, shape):
        return jax.random.normal(self._next(), shape, dtype=jnp.bfloat16)
    def randint(self, lo, hi, shape):
        return jax.random.randint(self._next(), shape, lo, hi, dtype=jnp.int32)
    def uniform(self, shape, lo=0.0, hi=1.0):
        return jax.random.uniform(self._next(), shape, jnp.bfloat16, lo, hi)
    def permutation(self, n):
        return jax.random.permutation(self._next(), n)


kernel_name = 'gated_mix__sliding_local_dilated__glu_gated_geglu__prompt'

def setup_inputs():
    _rng = _Rng(jax.random.key(int.from_bytes(__import__("os").urandom(4), "little")))
    _w = (lambda a: (lambda t: t.astype(jnp.bfloat16) if jnp.issubdtype(t.dtype, jnp.floating) else t)(jnp.asarray(a)))
    def _A_setup():
        B, S, D = 1, 2048, 1024
        return {
            "x": _w((lambda *s: _rng.normal(s) * 0.05)(B, S, D)),
            "wqkv": _w((lambda *s: _rng.normal(s) * 0.05)(D, 3 * D)),
            "wo": _w((lambda *s: _rng.normal(s) * 0.05)(D, D)),
        }
    _A_in = _A_setup()

    def _B_setup():
        B, S, Dm, Df = 1, 2048, 1024, 3584
        return {
            "x": _w((lambda *s: _rng.normal(s) * 0.05)(B, S, Dm)),
            "w_gate": _w((lambda *s: _rng.normal(s) * 0.05)(Dm, Df) * (Dm ** -0.5)),
            "w_up": _w((lambda *s: _rng.normal(s) * 0.05)(Dm, Df) * (Dm ** -0.5)),
            "w_down": _w((lambda *s: _rng.normal(s) * 0.05)(Df, Dm) * (Df ** -0.5)),
        }
    _B_in = _B_setup()

    return {
        "A_x": _A_in["x"],
        "A_wqkv": _A_in["wqkv"],
        "A_wo": _A_in["wo"],
        "B_x": _B_in["x"],
        "B_w_gate": _B_in["w_gate"],
        "B_w_up": _B_in["w_up"],
        "B_w_down": _B_in["w_down"],
        "gate_w": _w((lambda *s: _rng.normal(s) * 0.05)(1024)),
    }

def reference(A_x, A_wqkv, A_wo, B_x, B_w_gate, B_w_up, B_w_down, gate_w):
    def _A_ref(x, wqkv, wo):
        B, S, D = x.shape
        H = 32; Dh = D // H
        W, dil = 8, 2
        qkv = (lambda x, *d: x.transpose(*d))((x @ wqkv).reshape(B, S, 3, H, Dh), 2, 0, 3, 1, 4)
        q, k, v = qkv[0], qkv[1], qkv[2]
        scale = Dh ** -0.5
        pos = jnp.arange(S)
        off = jnp.arange(W) * dil
        idx = pos[:, None] - off[None, :]
        mask = idx >= 0
        idx_c = jnp.where(mask, idx, 0).reshape(-1)
        kg = k[:, :, idx_c, :].reshape(B, H, S, W, Dh)
        vg = v[:, :, idx_c, :].reshape(B, H, S, W, Dh)
        logits = jnp.einsum("bhsd,bhswd->bhsw", q, kg) * scale
        logits = jnp.where(mask[None, None, :, :], logits, -1e9)
        attn = _softmax(logits, axis=-1)
        o = jnp.einsum("bhsw,bhswd->bhsd", attn, vg)
        return (lambda x, *d: x.transpose(*d))(o, 0, 2, 1, 3).reshape(B, S, D) @ wo

    def _B_ref(x, w_gate, w_up, w_down):
        g = jnp.einsum("bsd,df->bsf", x, w_gate)
        u = jnp.einsum("bsd,df->bsf", x, w_up)
        h = _gelu(g) * u
        return jnp.einsum("bsf,fd->bsd", h, w_down)

    x = A_x
    g = _sigmoid((x * gate_w).sum(-1, keepdims=True))
    a = _A_ref(x, A_wqkv, A_wo)
    b = _B_ref(x, B_w_gate, B_w_up, B_w_down)
    return g * a + (1 - g) * b
```

```python
import jax
import jax.numpy as jnp
from jax import lax
from jax.experimental import pallas as pl
from jax.experimental.pallas import tpu as pltpu

S = 2048
D = 1024
F = 3584
H = 32
DH = 32
W = 8
DIL = 2
HALO = 16
LANES = 128
NCB = D // LANES

TM = 256
NA = S // TM
NB = S // TM
FC = 512
PAIR = 2 * LANES
NPAIR = 3 * D // PAIR

_NT = (((1,), (1,)), ((), ()))

SEM_AX0, SEM_AXR, SEM_GW, SEM_WO, SEM_BX, SEM_WG, SEM_WU, SEM_WD = range(8)
SEM_WQ = 8
NSEM = SEM_WQ + NPAIR


def _perm_matrix():
    r = lax.broadcasted_iota(jnp.int32, (LANES, LANES), 0)
    m = lax.broadcasted_iota(jnp.int32, (LANES, LANES), 1)
    src = ((r % 8) // 2) * 32 + (r // 8) * 2 + (r % 2)
    return jnp.where(m == src, 1.0, 0.0).astype(jnp.bfloat16)


def _store_pair(dst_ref, row0, out0, out1):
    comb = jnp.concatenate(
        [out0.reshape(16, 8, D), out1.reshape(16, 8, D)], axis=1
    ).astype(jnp.bfloat16)
    for dd in range(16):
        start = pl.multiple_of(row0 + dd * 64, 16)
        dst_ref[pl.ds(start, 16), :] = comb[dd]


def _attention_rows(qkv, r0, rg, row_in_tile_masked, step_row0):
    base = r0 + HALO + 8 * rg
    q = [qkv[j, pl.ds(base, 8), :] for j in range(NCB)]
    lane = lax.broadcasted_iota(jnp.int32, (8, LANES), 1)
    odd = (lane % 2) == 1
    scale = DH ** -0.5
    logits = []
    for w in range(W):
        s = None
        for j in range(NCB):
            t = q[j] * qkv[NCB + j, pl.ds(base - DIL * w, 8), :]
            s = t if s is None else s + t
        s = s + pltpu.roll(s, 64, 1)
        s = s + pltpu.roll(s, 1, 1)
        s = jnp.where(odd, s, pltpu.roll(s, LANES - 1, 1))
        s = s * scale
        if row_in_tile_masked and w > 0:
            row = step_row0 + 8 * rg + lax.broadcasted_iota(jnp.int32, (8, LANES), 0)
            s = jnp.where(row >= DIL * w, s, -1e9)
        logits.append(s)
    m = logits[0]
    for w in range(1, W):
        m = jnp.maximum(m, logits[w])
    p = [jnp.exp(s - m) for s in logits]
    den = p[0]
    for w in range(1, W):
        den = den + p[w]
    inv = 1.0 / den
    outs = []
    for j in range(NCB):
        o = None
        for w in range(W):
            t = p[w] * qkv[2 * NCB + j, pl.ds(base - DIL * w, 8), :]
            o = t if o is None else o + t
        outs.append(o * inv)
    return outs


def _kernel(ax_hbm, wqkv_hbm, wo_hbm, bx_hbm, wg_hbm, wu_hbm, wd_hbm, gw_hbm,
            out_ref,
            ax, bx, wraw, wt, woraw, wop, wg, wu, wd, gw, qkv, osc, sems):
    step = pl.program_id(0)

    def cp_wq(p):
        return pltpu.make_async_copy(
            wqkv_hbm.at[:, pl.ds(p * PAIR, PAIR)], wraw.at[p], sems.at[SEM_WQ + p])

    cp_ax0 = pltpu.make_async_copy(
        ax_hbm.at[pl.ds(0, TM), :], ax.at[pl.ds(0, TM), :], sems.at[SEM_AX0])
    cp_axr = pltpu.make_async_copy(
        ax_hbm.at[pl.ds(TM, S - TM), :], ax.at[pl.ds(TM, S - TM), :], sems.at[SEM_AXR])
    cp_gw = pltpu.make_async_copy(gw_hbm, gw, sems.at[SEM_GW])
    cp_wo = pltpu.make_async_copy(wo_hbm, woraw, sems.at[SEM_WO])
    cp_bx = pltpu.make_async_copy(bx_hbm, bx, sems.at[SEM_BX])
    cp_wg = pltpu.make_async_copy(wg_hbm, wg, sems.at[SEM_WG])
    cp_wu = pltpu.make_async_copy(wu_hbm, wu, sems.at[SEM_WU])
    cp_wd = pltpu.make_async_copy(wd_hbm, wd, sems.at[SEM_WD])

    @pl.when(step == 0)
    def _prologue():
        for p in range(NPAIR):
            cp_wq(p).start()
        cp_ax0.start()
        cp_axr.start()
        cp_gw.start()
        cp_wo.start()
        cp_wg.start()
        cp_wu.start()
        cp_wd.start()
        cp_bx.start()
        qkv[:, 0:HALO, :] = jnp.zeros((3 * NCB, HALO, LANES), jnp.float32)
        perm = _perm_matrix()

        def body(p, carry):
            cp_wq(p).wait()
            out0 = lax.dot_general(perm, wraw[p, :, 0:LANES], _NT,
                                   preferred_element_type=jnp.float32)
            out1 = lax.dot_general(perm, wraw[p, :, LANES:PAIR], _NT,
                                   preferred_element_type=jnp.float32)
            row0 = (p // 4) * D + (p % 4) * 16
            _store_pair(wt, row0, out0, out1)
            return carry

        lax.fori_loop(0, NPAIR, body, 0)
        cp_ax0.wait()

    @pl.when(step == 1)
    def _():
        cp_axr.wait()

    @pl.when(step < NA)
    def _phase_a():
        r0 = pl.multiple_of(step * TM, TM)
        x = ax[pl.ds(r0, TM), :]
        res = lax.dot_general(x, wt[...], _NT, preferred_element_type=jnp.float32)
        for jj in range(3 * NCB):
            qkv[jj, pl.ds(r0 + HALO, TM), :] = res[:, jj * LANES:(jj + 1) * LANES]

    @pl.when(step == NA)
    def _mid():
        cp_gw.wait()
        cp_wo.wait()
        perm = _perm_matrix()

        def body(pp, carry):
            b0 = pl.multiple_of(pp * PAIR, PAIR)
            out0 = jnp.dot(perm, woraw[pl.ds(b0, LANES), :],
                           preferred_element_type=jnp.float32)
            out1 = jnp.dot(perm, woraw[pl.ds(b0 + LANES, LANES), :],
                           preferred_element_type=jnp.float32)
            _store_pair(wop, pp * 16, out0, out1)
            return carry

        lax.fori_loop(0, 4, body, 0)
        cp_wg.wait()
        cp_wu.wait()
        cp_wd.wait()
        cp_bx.wait()

    @pl.when(step >= NA)
    def _phase_b():
        r0 = pl.multiple_of((step - NA) * TM, TM)
        for rg in range(TM // 8):
            outs = _attention_rows(qkv, r0, rg, rg < 2, r0)
            for j in range(NCB):
                osc[8 * rg:8 * rg + 8, j * LANES:(j + 1) * LANES] = outs[j].astype(jnp.bfloat16)
        x = bx[pl.ds(r0, TM), :]
        acc = None
        for c in range(F // FC):
            g = jnp.dot(x, wg[:, c * FC:(c + 1) * FC], preferred_element_type=jnp.float32)
            u = jnp.dot(x, wu[:, c * FC:(c + 1) * FC], preferred_element_type=jnp.float32)
            h = (jax.nn.gelu(g, approximate=True) * u).astype(jnp.bfloat16)
            d = jnp.dot(h, wd[c * FC:(c + 1) * FC, :], preferred_element_type=jnp.float32)
            acc = d if acc is None else acc + d
        a = jnp.dot(osc[...], wop[...], preferred_element_type=jnp.float32)
        xa = ax[pl.ds(r0, TM), :].astype(jnp.float32)
        glogit = jnp.sum(xa * gw[...].astype(jnp.float32), axis=-1, keepdims=True)
        gate = jax.nn.sigmoid(glogit)
        out_ref[...] = (gate * a + (1.0 - gate) * acc).astype(out_ref.dtype)


@jax.jit
def pallas_gated_mix__sliding_local_dilated__glu_gated_geglu__prompt_kernel(
    A_x: jax.Array,
    A_wqkv: jax.Array,
    A_wo: jax.Array,
    B_x: jax.Array,
    B_w_gate: jax.Array,
    B_w_up: jax.Array,
    B_w_down: jax.Array,
    gate_w: jax.Array,
):
    bf16 = jnp.bfloat16
    any_spec = pl.BlockSpec(memory_space=pl.ANY)
    out = pl.pallas_call(
        _kernel,
        grid=(NA + NB,),
        in_specs=[any_spec] * 8,
        out_specs=pl.BlockSpec((TM, D), lambda s: (jnp.maximum(s - NA, 0), 0)),
        out_shape=jax.ShapeDtypeStruct((S, D), bf16),
        scratch_shapes=[
            pltpu.VMEM((S, D), bf16),
            pltpu.VMEM((S, D), bf16),
            pltpu.VMEM((NPAIR, D, PAIR), bf16),
            pltpu.VMEM((3 * D, D), bf16),
            pltpu.VMEM((D, D), bf16),
            pltpu.VMEM((D, D), bf16),
            pltpu.VMEM((D, F), bf16),
            pltpu.VMEM((D, F), bf16),
            pltpu.VMEM((F, D), bf16),
            pltpu.VMEM((1, D), bf16),
            pltpu.VMEM((3 * NCB, HALO + S, LANES), jnp.float32),
            pltpu.VMEM((TM, D), bf16),
            pltpu.SemaphoreType.DMA((NSEM,)),
        ],
        compiler_params=pltpu.CompilerParams(
            dimension_semantics=("arbitrary",),
            vmem_limit_bytes=120 * 1024 * 1024,
        ),
    )(A_x.reshape(S, D), A_wqkv, A_wo, B_x.reshape(S, D), B_w_gate, B_w_up,
      B_w_down, gate_w.reshape(1, D))
    return out.reshape(1, S, D)
```

```python
import jax
import jax.numpy as jnp
from jax import lax
from jax.experimental import pallas as pl
from jax.experimental.pallas import tpu as pltpu
CFG = {'dep': 2, 'fc': 256}

S = 2048
D = 1024
F = 3584
H = 32
DH = 32
W = 8
DIL = 2
HALO = 16
LANES = 128
NCB = D // LANES

TM = 256
NA = S // TM
NB = S // TM
FC = CFG.get('fc', 512)
PAIR = 2 * LANES
NPAIR = 3 * D // PAIR

_NT = (((1,), (1,)), ((), ()))

SEM_AX0, SEM_AXR, SEM_GW, SEM_BX, SEM_WG, SEM_WU, SEM_WD = range(7)
SEM_WO = 7
SEM_WQ = 8
NSEM = SEM_WQ + NPAIR


def _perm_matrix():
    r = lax.broadcasted_iota(jnp.int32, (LANES, LANES), 0)
    m = lax.broadcasted_iota(jnp.int32, (LANES, LANES), 1)
    src = ((r % 8) // 2) * 32 + (r // 8) * 2 + (r % 2)
    return jnp.where(m == src, 1.0, 0.0).astype(jnp.bfloat16)


def _store_pair(dst_ref, row0, out0, out1):
    comb = jnp.concatenate(
        [out0.reshape(16, 8, D), out1.reshape(16, 8, D)], axis=1
    ).astype(jnp.bfloat16)
    for dd in range(16):
        start = pl.multiple_of(row0 + dd * 64, 16)
        dst_ref[pl.ds(start, 16), :] = comb[dd]


def _attention_rows(win, rg, row0):
    base = HALO + 8 * rg
    q = [win[j, base:base + 8, :] for j in range(NCB)]
    lane = lax.broadcasted_iota(jnp.int32, (8, LANES), 1)
    odd = (lane % 2) == 1
    scale = DH ** -0.5
    logits = []
    for w in range(W):
        lo = base - DIL * w
        s = None
        for j in range(NCB):
            t = q[j] * win[NCB + j, lo:lo + 8, :]
            s = t if s is None else s + t
        s = s + pltpu.roll(s, 64, 1)
        s = s + pltpu.roll(s, 1, 1)
        s = jnp.where(odd, s, pltpu.roll(s, LANES - 1, 1))
        s = s * scale
        if 8 * rg < DIL * w:
            row = row0 + 8 * rg + lax.broadcasted_iota(jnp.int32, (8, LANES), 0)
            s = jnp.where(row >= DIL * w, s, -1e9)
        logits.append(s)
    m = logits[0]
    for w in range(1, W):
        m = jnp.maximum(m, logits[w])
    p = [jnp.exp(s - m) for s in logits]
    den = p[0]
    for w in range(1, W):
        den = den + p[w]
    inv = 1.0 / den
    pn = [pw * inv for pw in p]
    outs = []
    for j in range(NCB):
        idx = 2 * (4 * j + lane // DH)
        o = None
        for w in range(W):
            lo = base - DIL * w
            t = jnp.take_along_axis(pn[w], idx, axis=1) * win[2 * NCB + j, lo:lo + 8, :]
            o = t if o is None else o + t
        outs.append(o)
    return outs


def _kernel(ax_hbm, wqkv_hbm, wo_hbm, bx_hbm, wg_hbm, wu_hbm, wd_hbm, gw_hbm,
            out_ref,
            ax, bx, wraw, wt, wo, wg, wu, wd, gw, qkv, win, osc, flag, sems):
    step = pl.program_id(0)

    def cp_wq(p):
        return pltpu.make_async_copy(
            wqkv_hbm.at[:, pl.ds(p * PAIR, PAIR)], wraw.at[p], sems.at[SEM_WQ + p])

    cp_wo = pltpu.make_async_copy(wo_hbm, wo, sems.at[SEM_WO])
    cp_ax0 = pltpu.make_async_copy(
        ax_hbm.at[pl.ds(0, TM), :], ax.at[pl.ds(0, TM), :], sems.at[SEM_AX0])
    cp_axr = pltpu.make_async_copy(
        ax_hbm.at[pl.ds(TM, S - TM), :], ax.at[pl.ds(TM, S - TM), :], sems.at[SEM_AXR])
    cp_gw = pltpu.make_async_copy(gw_hbm, gw, sems.at[SEM_GW])
    cp_bx = pltpu.make_async_copy(bx_hbm, bx, sems.at[SEM_BX])
    cp_wg = pltpu.make_async_copy(wg_hbm, wg, sems.at[SEM_WG])
    cp_wu = pltpu.make_async_copy(wu_hbm, wu, sems.at[SEM_WU])
    cp_wd = pltpu.make_async_copy(wd_hbm, wd, sems.at[SEM_WD])

    @pl.when(step == 0)
    @jax.named_scope("prologue")
    def _prologue():
        for p in range(4):
            cp_wq(p).start()
        cp_ax0.start()
        for p in range(4, NPAIR):
            cp_wq(p).start()
        cp_axr.start()
        cp_gw.start()
        cp_wo.start()
        cp_wg.start()
        cp_wu.start()
        cp_wd.start()
        cp_bx.start()
        flag[0] = 0
        win[:, 0:HALO, :] = jnp.zeros((3 * NCB, HALO, LANES), jnp.float32)
        perm = _perm_matrix()
        PW = CFG.get('pw', 2)

        def store_tile0(jj, blk):
            win[jj, HALO:HALO + TM, :] = blk
            qkv[jj, TM - HALO:TM, :] = blk[TM - HALO:, :]

        def body(t, carry):
            for pp in range(4):
                p = t * 4 + pp
                if pp % PW == 0:
                    for k in range(PW):
                        cp_wq(p + k).wait()
                out0 = lax.dot_general(perm, wraw[p, :, 0:LANES], _NT,
                                       preferred_element_type=jnp.float32)
                out1 = lax.dot_general(perm, wraw[p, :, LANES:PAIR], _NT,
                                       preferred_element_type=jnp.float32)
                _store_pair(wt, t * D + pp * 16, out0, out1)

            @pl.when(t == 0)
            def _():
                cp_ax0.wait()

            x = ax[0:TM, :]
            res = lax.dot_general(x, wt[pl.ds(pl.multiple_of(t * D, D), D), :], _NT,
                                  preferred_element_type=jnp.float32)
            for j in range(NCB):
                store_tile0(t * NCB + j, res[:, j * LANES:(j + 1) * LANES])
            return carry

        lax.fori_loop(0, 2, body, 0)

        VG = CFG.get('vg', 2)

        def vbody(i, carry):
            x = ax[0:TM, :]
            for k in range(VG):
                cp_wq(8 + i * VG + k).wait()
            for k in range(VG):
                c = i * VG + k
                res = jnp.dot(x, wraw[8 + c], preferred_element_type=jnp.float32)
                store_tile0(2 * NCB + 2 * c, res[:, 0:LANES])
                store_tile0(2 * NCB + 2 * c + 1, res[:, LANES:PAIR])
            return carry

        lax.fori_loop(0, 4 // VG, vbody, 0)

    @pl.when(step == 1)
    def _():
        cp_axr.wait()

    @pl.when(jnp.logical_and(step >= 1, step < NA))
    @jax.named_scope("phase_a")
    def _phase_a():
        r0 = pl.multiple_of(step * TM, TM)

        x = ax[pl.ds(r0, TM), :]
        res = lax.dot_general(x, wt[...], _NT, preferred_element_type=jnp.float32)
        for jj in range(2 * NCB):
            qkv[jj, pl.ds(r0, TM), :] = res[:, jj * LANES:(jj + 1) * LANES]
        for c in range(4):
            res = jnp.dot(x, wraw[8 + c], preferred_element_type=jnp.float32)
            qkv[2 * NCB + 2 * c, pl.ds(r0, TM), :] = res[:, 0:LANES]
            qkv[2 * NCB + 2 * c + 1, pl.ds(r0, TM), :] = res[:, LANES:PAIR]

    @pl.when(step == NA)
    def _():
        cp_wo.wait()
        cp_gw.wait()
        cp_wg.wait()
        cp_wu.wait()
        cp_wd.wait()
        cp_bx.wait()

    @pl.when(step >= NA)
    @jax.named_scope("phase_b")
    def _phase_b():
        r0 = pl.multiple_of((step - NA) * TM, TM)
        never = flag[0] != 0
        nrg = TM // 8
        nblk = F // LANES

        def attn(rg):
            outs = _attention_rows(win, rg, r0)
            for j in range(NCB):
                osc[8 * rg:8 * rg + 8, j * LANES:(j + 1) * LANES] = outs[j].astype(jnp.bfloat16)
            return outs[NCB - 1]

        dep_mode = CFG.get('dep', 1)
        x = bx[pl.ds(r0, TM), :]
        acc = None
        bpc = FC // LANES
        if dep_mode == 0:
            for rg in range(nrg):
                attn(rg)
        if dep_mode in (0, 1):
            first_blk = CFG.get('dep_first', 2)
            last_blk = CFG.get('dep_last', nblk - 1)
            deadline = {}
            for rg in range(nrg):
                n = first_blk + rg * (last_blk - first_blk + 1) // nrg
                deadline.setdefault(n, []).append(rg)
            for c in range(F // FC):
                g = jnp.dot(x, wg[:, c * FC:(c + 1) * FC], preferred_element_type=jnp.float32)
                u = jnp.dot(x, wu[:, c * FC:(c + 1) * FC], preferred_element_type=jnp.float32)
                if dep_mode:
                    blocks = []
                    for b in range(bpc):
                        gb = g[:, b * LANES:(b + 1) * LANES]
                        rgs = deadline.get(c * bpc + b, [])
                        if rgs:
                            rows = []
                            for i, rg in enumerate(rgs):
                                dep = attn(rg)
                                rows.append(jnp.where(never, dep, gb[8 * i:8 * i + 8, :]))
                            rows.append(gb[8 * len(rgs):, :])
                            gb = jnp.concatenate(rows, axis=0)
                        blocks.append(gb)
                    g = jnp.concatenate(blocks, axis=1)
                h = (jax.nn.gelu(g, approximate=True) * u).astype(jnp.bfloat16)
                d = jnp.dot(h, wd[c * FC:(c + 1) * FC, :], preferred_element_type=jnp.float32)
                acc = d if acc is None else acc + d
        elif dep_mode == 2:
            GW = CFG.get('gw', 1)
            nslots = 2 * nblk // GW
            s_first = CFG.get('s_first', 2)
            s_last = CFG.get('s_last', nslots - 1)
            deadline = {}
            for rg in range(nrg):
                n = s_first + rg * (s_last - s_first + 1) // nrg
                deadline.setdefault(n, []).append(rg)

            def lhs(slot):
                rgs = deadline.get(slot, [])
                if not rgs:
                    return x
                tiles = []
                for i, rg in enumerate(rgs):
                    dep = attn(rg)
                    xt = pltpu.bitcast(x[0:16, i * LANES:(i + 1) * LANES], jnp.float32)
                    tiles.append(pltpu.bitcast(jnp.where(never, dep, xt), jnp.bfloat16))
                top = jnp.concatenate(tiles + [x[0:16, len(rgs) * LANES:]], axis=1)
                return jnp.concatenate([top, x[16:, :]], axis=0)

            for c in range(F // FC):
                hs = []
                for b in range(0, bpc, GW):
                    n = c * bpc + b
                    cols = slice(n * LANES, (n + GW) * LANES)
                    g = jnp.dot(lhs(2 * (n // GW)), wg[:, cols], preferred_element_type=jnp.float32)
                    u = jnp.dot(lhs(2 * (n // GW) + 1), wu[:, cols], preferred_element_type=jnp.float32)
                    hs.append((jax.nn.gelu(g, approximate=True) * u).astype(jnp.bfloat16))
                h = jnp.concatenate(hs, axis=1)
                d = jnp.dot(h, wd[c * FC:(c + 1) * FC, :], preferred_element_type=jnp.float32)
                acc = d if acc is None else acc + d

        rn = pl.multiple_of(jnp.minimum(step - NA + 1, NB - 1) * TM, TM)
        for jj in range(3 * NCB):
            if jj < NCB:
                win[jj, HALO:, :] = qkv[jj, pl.ds(rn, TM), :]
            else:
                win[jj] = qkv[jj, pl.ds(pl.multiple_of(rn - HALO, 8), TM + HALO), :]

        xa = ax[pl.ds(r0, TM), :].astype(jnp.float32)
        gwv = gw[...].astype(jnp.float32).reshape(1, D)
        glogit = jnp.sum(xa * gwv, axis=-1, keepdims=True)
        gate = jax.nn.sigmoid(glogit)
        a = jnp.dot(osc[...], wo[...], preferred_element_type=jnp.float32)
        out_ref[...] = (gate * a + (1.0 - gate) * acc).astype(out_ref.dtype)


@jax.jit
def pallas_gated_mix__sliding_local_dilated__glu_gated_geglu__prompt_kernel(
    A_x, A_wqkv, A_wo, B_x, B_w_gate, B_w_up, B_w_down, gate_w,
):
    bf16 = jnp.bfloat16
    any_spec = pl.BlockSpec(memory_space=pl.ANY)
    out = pl.pallas_call(
        _kernel,
        grid=(NA + NB,),
        in_specs=[any_spec] * 8,
        out_specs=pl.BlockSpec((TM, D), lambda s: (jnp.maximum(s - NA, 0), 0)),
        out_shape=jax.ShapeDtypeStruct((S, D), bf16),
        scratch_shapes=[
            pltpu.VMEM((S, D), bf16),
            pltpu.VMEM((S, D), bf16),
            pltpu.VMEM((NPAIR, D, PAIR), bf16),
            pltpu.VMEM((2 * D, D), bf16),
            pltpu.VMEM((D, D), bf16),
            pltpu.VMEM((D, F), bf16),
            pltpu.VMEM((D, F), bf16),
            pltpu.VMEM((F, D), bf16),
            pltpu.VMEM((D,), bf16),
            pltpu.VMEM((3 * NCB, S, LANES), jnp.float32),
            pltpu.VMEM((3 * NCB, HALO + TM, LANES), jnp.float32),
            pltpu.VMEM((TM, D), bf16),
            pltpu.SMEM((1,), jnp.int32),
            pltpu.SemaphoreType.DMA((NSEM,)),
        ],
        compiler_params=pltpu.CompilerParams(
            dimension_semantics=("arbitrary",),
            vmem_limit_bytes=120 * 1024 * 1024,
        ),
    )(A_x.reshape(S, D), A_wqkv, A_wo, B_x.reshape(S, D), B_w_gate, B_w_up,
      B_w_down, gate_w)
    return out.reshape(1, S, D)
```

```python
import contextlib
import jax
import jax.numpy as jnp
from jax import lax
from jax.experimental import pallas as pl
from jax.experimental.pallas import tpu as pltpu
CFG = {'gate_a': 0, 'v_first': 1, 'og': 8, 'wdma': 0, 's_first': 3, 's_last': 50, 'scopes': 0}

S = 2048
D = 1024
F = 3584
H = 32
DH = 32
W = 8
DIL = 2
HALO = 16
LANES = 128
NCB = D // LANES

TM = 256
NT_ = S // TM
FC = CFG.get('fc', 256)
PAIR = 2 * LANES
NPAIR = 3 * D // PAIR

_NT = (((1,), (1,)), ((), ()))

SEM_AX0, SEM_AXR, SEM_GW, SEM_BX, SEM_WG, SEM_WU, SEM_WD, SEM_WO = range(8)
SEM_WQ = 8
SEM_OUT = SEM_WQ + NPAIR
SEM_WIN = SEM_OUT + 2 * CFG.get('og', 1)
NSEM = SEM_WIN + 1


def _scope(name):
    return jax.named_scope(name) if CFG.get('scopes', 1) else contextlib.nullcontext()


def _perm_matrix():
    r = lax.broadcasted_iota(jnp.int32, (LANES, LANES), 0)
    m = lax.broadcasted_iota(jnp.int32, (LANES, LANES), 1)
    src = ((r % 8) // 2) * 32 + (r // 8) * 2 + (r % 2)
    return jnp.where(m == src, 1.0, 0.0).astype(jnp.bfloat16)


def _store_pair(dst_ref, row0, out0, out1):
    comb = jnp.concatenate(
        [out0.reshape(16, 8, D), out1.reshape(16, 8, D)], axis=1
    ).astype(jnp.bfloat16)
    for dd in range(16):
        start = pl.multiple_of(row0 + dd * 64, 16)
        dst_ref[pl.ds(start, 16), :] = comb[dd]


def _attention_rows(win, rg, row0):
    base = HALO + 8 * rg
    q = [win[j, base:base + 8, :] for j in range(NCB)]
    lane = lax.broadcasted_iota(jnp.int32, (8, LANES), 1)
    odd = (lane % 2) == 1
    scale = DH ** -0.5
    logits = []
    for w in range(W):
        lo = base - DIL * w
        s = None
        for j in range(NCB):
            t = q[j] * win[NCB + j, lo:lo + 8, :]
            s = t if s is None else s + t
        s = s + pltpu.roll(s, 64, 1)
        s = s + pltpu.roll(s, 1, 1)
        s = jnp.where(odd, s, pltpu.roll(s, LANES - 1, 1))
        s = s * scale
        if 8 * rg < DIL * w:
            row = row0 + 8 * rg + lax.broadcasted_iota(jnp.int32, (8, LANES), 0)
            s = jnp.where(row >= DIL * w, s, -1e9)
        logits.append(s)
    m = logits[0]
    for w in range(1, W):
        m = jnp.maximum(m, logits[w])
    p = [jnp.exp(s - m) for s in logits]
    den = p[0]
    for w in range(1, W):
        den = den + p[w]
    inv = 1.0 / den
    pn = [pw * inv for pw in p]
    outs = []
    for j in range(NCB):
        idx = 2 * (4 * j + lane // DH)
        o = None
        for w in range(W):
            lo = base - DIL * w
            t = jnp.take_along_axis(pn[w], idx, axis=1) * win[2 * NCB + j, lo:lo + 8, :]
            o = t if o is None else o + t
        outs.append(o)
    return outs


WDMA = CFG.get('wdma', 1)
PK = 0 if WDMA else CFG.get('pk', 1)


def _pack(blk):
    return pltpu.bitcast(blk.astype(jnp.bfloat16), jnp.uint32)


def _unpack(words):
    return pltpu.bitcast(words, jnp.bfloat16).astype(jnp.float32)


def _put(qkv, jj, r0, blk):
    n = blk.shape[0]
    if PK:
        start = r0 // 2 if isinstance(r0, int) else pl.multiple_of(r0 // 2, 8)
        qkv[jj, pl.ds(start, n // 2), :] = _pack(blk)
    else:
        qkv[jj, pl.ds(r0, n), :] = blk


def _get(qkv, jj, r0, n):
    if PK:
        return _unpack(qkv[jj, pl.ds(pl.multiple_of(r0 // 2, 8), n // 2), :])
    return qkv[jj, pl.ds(pl.multiple_of(r0, 8), n), :]


def _gate(x, gw):
    gwv = gw[...].astype(jnp.float32).reshape(1, D)
    glogit = jnp.sum(x.astype(jnp.float32) * gwv, axis=-1, keepdims=True)
    return jnp.broadcast_to(jax.nn.sigmoid(glogit), (x.shape[0], LANES))


def _kernel(ax_hbm, wqkv_hbm, wo_hbm, bx_hbm, wg_hbm, wu_hbm, wd_hbm, gw_hbm,
            out_hbm,
            ax, bx, wraw, wt, wo, wg, wu, wd, gw, qkv, win, gates, osc, obuf, flag, sems):

    def cp_wq(p):
        return pltpu.make_async_copy(
            wqkv_hbm.at[:, pl.ds(p * PAIR, PAIR)], wraw.at[p], sems.at[SEM_WQ + p])

    OG = CFG.get('og', 1)
    OW = D // OG

    def cp_out(i, g):
        slot = i % 2
        return pltpu.make_async_copy(
            obuf.at[slot, :, pl.ds(g * OW, OW)],
            out_hbm.at[pl.ds(pl.multiple_of(i * TM, TM), TM), pl.ds(g * OW, OW)],
            sems.at[SEM_OUT + slot * OG + g])

    def cp_win(i):
        start = pl.multiple_of(i * TM - HALO, 8)
        return pltpu.make_async_copy(
            qkv.at[:, pl.ds(start, TM + HALO), :], win, sems.at[SEM_WIN])

    cp_wo = pltpu.make_async_copy(wo_hbm, wo, sems.at[SEM_WO])
    cp_ax0 = pltpu.make_async_copy(
        ax_hbm.at[pl.ds(0, TM), :], ax.at[pl.ds(0, TM), :], sems.at[SEM_AX0])
    cp_axr = pltpu.make_async_copy(
        ax_hbm.at[pl.ds(TM, S - TM), :], ax.at[pl.ds(TM, S - TM), :], sems.at[SEM_AXR])
    cp_gw = pltpu.make_async_copy(gw_hbm, gw, sems.at[SEM_GW])
    cp_bx = pltpu.make_async_copy(bx_hbm, bx, sems.at[SEM_BX])
    cp_wg = pltpu.make_async_copy(wg_hbm, wg, sems.at[SEM_WG])
    cp_wu = pltpu.make_async_copy(wu_hbm, wu, sems.at[SEM_WU])
    cp_wd = pltpu.make_async_copy(wd_hbm, wd, sems.at[SEM_WD])

    gate_in_a = CFG.get('gate_a', 1)

    with _scope("prologue"):
        for p in range(4):
            cp_wq(p).start()
        cp_ax0.start()
        cp_gw.start()
        for p in range(4, NPAIR):
            cp_wq(p).start()
        cp_axr.start()
        cp_wo.start()
        cp_wg.start()
        cp_wu.start()
        cp_wd.start()
        cp_bx.start()
        flag[0] = 0
        win[:, 0:HALO, :] = jnp.zeros((3 * NCB, HALO, LANES), jnp.float32)
        perm = _perm_matrix()
        PW = CFG.get('pw', 2)

        def store_tile0(jj, blk):
            win[jj, HALO:HALO + TM, :] = blk
            _put(qkv, jj, TM - HALO, blk[TM - HALO:, :])

        def body(t, carry):
            for pp in range(4):
                p = t * 4 + pp
                if pp % PW == 0:
                    for k in range(PW):
                        cp_wq(p + k).wait()
                out0 = lax.dot_general(perm, wraw[p, :, 0:LANES], _NT,
                                       preferred_element_type=jnp.float32)
                out1 = lax.dot_general(perm, wraw[p, :, LANES:PAIR], _NT,
                                       preferred_element_type=jnp.float32)
                _store_pair(wt, t * D + pp * 16, out0, out1)

            @pl.when(t == 0)
            def _():
                cp_ax0.wait()
                cp_gw.wait()

            x = ax[0:TM, :]
            res = lax.dot_general(x, wt[pl.ds(pl.multiple_of(t * D, D), D), :], _NT,
                                  preferred_element_type=jnp.float32)
            for j in range(NCB):
                store_tile0(t * NCB + j, res[:, j * LANES:(j + 1) * LANES])
            return carry

        lax.fori_loop(0, 2, body, 0)

        VG = CFG.get('vg', 4)

        def vbody(i, carry):
            for k in range(VG):
                cp_wq(8 + i * VG + k).wait()
            x = ax[0:TM, :]
            for k in range(VG):
                c = i * VG + k
                res = jnp.dot(x, wraw[8 + c], preferred_element_type=jnp.float32)
                store_tile0(2 * NCB + 2 * c, res[:, 0:LANES])
                store_tile0(2 * NCB + 2 * c + 1, res[:, LANES:PAIR])
            if gate_in_a and VG == 4:
                gates[0:TM, :] = _gate(x, gw)
            return carry

        if VG == 4:
            vbody(0, 0)
        else:
            lax.fori_loop(0, 4 // VG, vbody, 0)
        cp_axr.wait()

    def phase_a(i, carry):
        with _scope("phase_a"):
            r0 = pl.multiple_of(i * TM, TM)
            x = ax[pl.ds(r0, TM), :]

            def qk():
                res = lax.dot_general(x, wt[...], _NT, preferred_element_type=jnp.float32)
                for jj in range(2 * NCB):
                    _put(qkv, jj, r0, res[:, jj * LANES:(jj + 1) * LANES])

            def v():
                for c in range(4):
                    res = jnp.dot(x, wraw[8 + c], preferred_element_type=jnp.float32)
                    _put(qkv, 2 * NCB + 2 * c, r0, res[:, 0:LANES])
                    _put(qkv, 2 * NCB + 2 * c + 1, r0, res[:, LANES:PAIR])

            if CFG.get('v_first', 0):
                v(); qk()
            else:
                qk(); v()
            if gate_in_a:
                gates[pl.ds(r0, TM), :] = _gate(x, gw)
        return carry

    lax.fori_loop(1, NT_, phase_a, 0)

    cp_wo.wait()
    cp_wg.wait()
    cp_wu.wait()
    cp_wd.wait()
    cp_bx.wait()

    def phase_b(i, carry):
        @pl.when(jnp.logical_and(i >= 2, not CFG.get('noout')))
        def _():
            for g in range(OG):
                cp_out(i - 2, g).wait()

        if WDMA:
            @pl.when(i >= 1)
            def _():
                cp_win(i).wait()

        with _scope("phase_b"):
            r0 = pl.multiple_of(i * TM, TM)
            never = flag[0] != 0
            nrg = TM // 8
            nblk = F // LANES

            def attn(rg):
                outs = _attention_rows(win, rg, r0)
                for j in range(NCB):
                    osc[8 * rg:8 * rg + 8, j * LANES:(j + 1) * LANES] = outs[j].astype(jnp.bfloat16)
                return outs[NCB - 1]

            dep_mode = CFG.get('dep', 2)
            x = bx[0:TM, :] if CFG.get('static_x') else bx[pl.ds(r0, TM), :]
            acc = None
            bpc = FC // LANES
            if dep_mode == 1:
                first_blk = CFG.get('dep_first', 2)
                last_blk = CFG.get('dep_last', nblk - 1)
                deadline = {}
                for rg in range(nrg):
                    n = first_blk + rg * (last_blk - first_blk + 1) // nrg
                    deadline.setdefault(n, []).append(rg)
                for c in range(F // FC):
                    g = jnp.dot(x, wg[:, c * FC:(c + 1) * FC], preferred_element_type=jnp.float32)
                    u = jnp.dot(x, wu[:, c * FC:(c + 1) * FC], preferred_element_type=jnp.float32)
                    blocks = []
                    for b in range(bpc):
                        gb = g[:, b * LANES:(b + 1) * LANES]
                        rgs = deadline.get(c * bpc + b, [])
                        if rgs:
                            rows = []
                            for k, rg in enumerate(rgs):
                                dep = attn(rg)
                                rows.append(jnp.where(never, dep, gb[8 * k:8 * k + 8, :]))
                            rows.append(gb[8 * len(rgs):, :])
                            gb = jnp.concatenate(rows, axis=0)
                        blocks.append(gb)
                    g = jnp.concatenate(blocks, axis=1)
                    h = (jax.nn.gelu(g, approximate=True) * u).astype(jnp.bfloat16)
                    d = jnp.dot(h, wd[c * FC:(c + 1) * FC, :], preferred_element_type=jnp.float32)
                    acc = d if acc is None else acc + d
            else:
                nslots = 2 * nblk
                s_first = CFG.get('s_first', 2)
                s_last = CFG.get('s_last', nslots - 1)
                deadline = {}
                for rg in range(nrg):
                    n = s_first + rg * (s_last - s_first + 1) // nrg
                    deadline.setdefault(n, []).append(rg)

                def lhs(slot):
                    rgs = deadline.get(slot, [])
                    if not rgs:
                        return x
                    tiles = []
                    for k, rg in enumerate(rgs):
                        dep = attn(rg)
                        xt = pltpu.bitcast(x[0:16, k * LANES:(k + 1) * LANES], jnp.float32)
                        tiles.append(pltpu.bitcast(jnp.where(never, dep, xt), jnp.bfloat16))
                    top = jnp.concatenate(tiles + [x[0:16, len(rgs) * LANES:]], axis=1)
                    return jnp.concatenate([top, x[16:, :]], axis=0)

                for c in range(F // FC):
                    hs = []
                    for b in range(bpc):
                        n = c * bpc + b
                        cols = slice(n * LANES, (n + 1) * LANES)
                        g = jnp.dot(lhs(2 * n), wg[:, cols], preferred_element_type=jnp.float32)
                        u = jnp.dot(lhs(2 * n + 1), wu[:, cols], preferred_element_type=jnp.float32)
                        hs.append((jax.nn.gelu(g, approximate=True) * u).astype(jnp.bfloat16))
                    h = jnp.concatenate(hs, axis=1)
                    d = jnp.dot(h, wd[c * FC:(c + 1) * FC, :], preferred_element_type=jnp.float32)
                    acc = d if acc is None else acc + d

            nxt = jnp.minimum(i + 1, NT_ - 1)
            if WDMA:
                cp_win(nxt).start()
            else:
                rn = pl.multiple_of(nxt * TM, TM)
                for jj in range(3 * NCB):
                    if jj < NCB:
                        win[jj, HALO:, :] = _get(qkv, jj, rn, TM)
                    else:
                        win[jj] = _get(qkv, jj, rn - HALO, TM + HALO)

            if gate_in_a:
                gate = gates[pl.ds(r0, TM), :]
            else:
                gate = _gate(ax[pl.ds(r0, TM), :], gw)
            a = jnp.dot(osc[...], wo[...], preferred_element_type=jnp.float32)
            slot = i % 2
            for cb in range(NCB):
                cols = slice(cb * LANES, (cb + 1) * LANES)
                obuf[slot, :, cols] = (gate * a[:, cols] + (1.0 - gate) * acc[:, cols]).astype(jnp.bfloat16)
                if ((cb + 1) * LANES) % OW == 0 and (cb + 1) * LANES < D:
                    cp_out(i, (cb + 1) * LANES // OW - 1).start()
        if not CFG.get('noout'):
            cp_out(i, OG - 1).start()
        return carry

    lax.fori_loop(0, NT_, phase_b, 0)
    if WDMA:
        cp_win(NT_ - 1).wait()
    for g in range(OG):
        cp_out(NT_ - 2, g).wait()
    for g in range(OG):
        cp_out(NT_ - 1, g).wait()


@jax.jit
def pallas_gated_mix__sliding_local_dilated__glu_gated_geglu__prompt_kernel(
    A_x, A_wqkv, A_wo, B_x, B_w_gate, B_w_up, B_w_down, gate_w,
):
    bf16 = jnp.bfloat16
    any_spec = pl.BlockSpec(memory_space=pl.ANY)
    out = pl.pallas_call(
        _kernel,
        in_specs=[any_spec] * 8,
        out_specs=any_spec,
        out_shape=jax.ShapeDtypeStruct((S, D), bf16),
        scratch_shapes=[
            pltpu.VMEM((S, D), bf16),
            pltpu.VMEM((S, D), bf16),
            pltpu.VMEM((NPAIR, D, PAIR), bf16),
            pltpu.VMEM((2 * D, D), bf16),
            pltpu.VMEM((D, D), bf16),
            pltpu.VMEM((D, F), bf16),
            pltpu.VMEM((D, F), bf16),
            pltpu.VMEM((F, D), bf16),
            pltpu.VMEM((D,), bf16),
            (pltpu.VMEM((3 * NCB, S // 2, LANES), jnp.uint32) if PK else pltpu.VMEM((3 * NCB, S, LANES), jnp.float32)),
            pltpu.VMEM((3 * NCB, HALO + TM, LANES), jnp.float32),
            pltpu.VMEM((S, LANES), jnp.float32),
            pltpu.VMEM((TM, D), bf16),
            pltpu.VMEM((2, TM, D), bf16),
            pltpu.SMEM((1,), jnp.int32),
            pltpu.SemaphoreType.DMA((NSEM,)),
        ],
        compiler_params=pltpu.CompilerParams(
            vmem_limit_bytes=120 * 1024 * 1024,
            disable_bounds_checks=bool(CFG.get('nochk', 1)),
            disable_semaphore_checks=bool(CFG.get('nochk', 1)),
        ),
    )(A_x.reshape(S, D), A_wqkv, A_wo, B_x.reshape(S, D), B_w_gate, B_w_up,
      B_w_down, gate_w)
    return out.reshape(1, S, D)
```

```python
import contextlib
import functools
import jax
import jax.numpy as jnp
from jax import lax
from jax.experimental import pallas as pl
from jax.experimental.pallas import tpu as pltpu
CFG = {'s_first': 3, 's_last': 52, 'rdelay': 3, 'padw': 8, 'scopes': 0}

S = 2048
D = 1024
F = 3584
H = 32
DH = 32
W = 8
DIL = 2
HALO = 16
LANES = 128
NCB = D // LANES

TM = 256
NT_ = S // TM
TA = CFG.get('ta', 448)
NA = (S - TM) // TA
assert TM + NA * TA == S
FC = CFG.get('fc', 256)
WC = 256
NWC = 3 * D // WC
BPC = WC // LANES

SEM_AX0, SEM_AXR, SEM_GW, SEM_BX, SEM_WG, SEM_WU, SEM_WD, SEM_WO, SEM_AX1 = range(9)
SEM_WQ = 9
SEM_OUT = SEM_WQ + NWC
OG = CFG.get('og', 8)
OW = D // OG
NSEM = SEM_OUT + 2 * OG

QSCALE = DH ** -0.5


def _scope(name):
    return jax.named_scope(name) if CFG.get('scopes', 1) else contextlib.nullcontext()


def _head_align(nat):
    rows = list(nat)
    lane = lax.broadcasted_iota(jnp.int32, rows[0].shape, 1)
    for s in range(3):
        shift = 4 << s
        low = (lane & shift) == 0
        for b in range(NCB):
            if b & (1 << s):
                continue
            b2 = b | (1 << s)
            lo_row, hi_row = rows[b], rows[b2]
            rows[b] = jnp.where(low, lo_row, pltpu.roll(hi_row, shift, 1))
            rows[b2] = jnp.where(low, pltpu.roll(lo_row, LANES - shift, 1), hi_row)
    return rows


def _attention_rows(win, rg, row0):
    base = HALO + 8 * rg
    q = [win[j, base:base + 8, :] for j in range(NCB)]
    lane = lax.broadcasted_iota(jnp.int32, (8, LANES), 1)
    logits = []
    for w in range(W):
        lo = base - DIL * w
        s = None
        for j in range(NCB):
            t = q[j] * win[NCB + j, lo:lo + 8, :]
            s = t if s is None else s + t
        s = s + pltpu.roll(s, 1, 1)
        s = s + pltpu.roll(s, 2, 1)
        if 8 * rg < DIL * w:
            row = row0 + 8 * rg + lax.broadcasted_iota(jnp.int32, (8, LANES), 0)
            s = jnp.where(row >= DIL * w, s, -1e9)
        logits.append(s)
    m = logits[0]
    for w in range(1, W):
        m = jnp.maximum(m, logits[w])
    p = [jnp.exp(s - m) for s in logits]
    den = p[0]
    for w in range(1, W):
        den = den + p[w]
    inv = 1.0 / den
    pn = [pw * inv for pw in p]
    outs = []
    for j in range(NCB):
        idx = (lane // DH) * DH + (4 * j + 3)
        o = None
        for w in range(W):
            lo = base - DIL * w
            t = jnp.take_along_axis(pn[w], idx, axis=1) * win[2 * NCB + j, lo:lo + 8, :]
            o = t if o is None else o + t
        outs.append(o)
    return outs


def _pack(blk):
    return pltpu.bitcast(blk.astype(jnp.bfloat16), jnp.uint32)


def _unpack(words):
    return pltpu.bitcast(words, jnp.bfloat16).astype(jnp.float32)


def _put(qkv, jj, r0, blk):
    start = (r0 + HALO) // 2
    if not isinstance(r0, int):
        start = pl.multiple_of(start, 8)
    qkv[jj, pl.ds(start, blk.shape[0] // 2), :] = _pack(blk)


def _refill(qkv, win, tile_row0, m):
    rows = slice(16 * m, 16 * m + 16)
    start = tile_row0 // 2 + 8 * m
    if not isinstance(start, int):
        start = pl.multiple_of(start, 8)
    vals = [_unpack(qkv[jj, pl.ds(start, 8), :]) for jj in range(3 * NCB)]
    qa = _head_align(vals[0:NCB])
    ka = _head_align(vals[NCB:2 * NCB])
    for j in range(NCB):
        win[j, rows, :] = qa[j] * QSCALE
        win[NCB + j, rows, :] = ka[j]
        win[2 * NCB + j, rows, :] = vals[2 * NCB + j]
    return ka[NCB - 1][0:8, :]


def _gate(x, gw):
    gwv = gw[...].astype(jnp.float32).reshape(1, D)
    glogit = jnp.sum(x.astype(jnp.float32) * gwv, axis=-1, keepdims=True)
    return jax.nn.sigmoid(glogit)


def _kernel(ax_hbm, wqkv_hbm, wo_hbm, bx_hbm, wg_hbm, wu_hbm, wd_hbm, gw_hbm,
            out_hbm,
            ax, bx, wq, wo, wg, wu, wd, gw, qkv, t0, win, osc, obuf, flag, sems):

    def cp_wq(p):
        return pltpu.make_async_copy(
            wqkv_hbm.at[:, pl.ds(p * WC, WC)], wq.at[p], sems.at[SEM_WQ + p])

    def cp_out(i, g):
        slot = i % 2
        return pltpu.make_async_copy(
            obuf.at[slot, :, pl.ds(g * OW, OW)],
            out_hbm.at[pl.ds(pl.multiple_of(i * TM, TM), TM), pl.ds(g * OW, OW)],
            sems.at[SEM_OUT + slot * OG + g])

    cp_wo = pltpu.make_async_copy(wo_hbm, wo, sems.at[SEM_WO])
    cp_ax0 = pltpu.make_async_copy(
        ax_hbm.at[pl.ds(0, TM), :], ax.at[pl.ds(0, TM), :], sems.at[SEM_AX0])
    cp_ax1 = pltpu.make_async_copy(
        ax_hbm.at[pl.ds(TM, TA), :], ax.at[pl.ds(TM, TA), :], sems.at[SEM_AX1])
    cp_axr = pltpu.make_async_copy(
        ax_hbm.at[pl.ds(TM + TA, S - TM - TA), :], ax.at[pl.ds(TM + TA, S - TM - TA), :], sems.at[SEM_AXR])
    cp_gw = pltpu.make_async_copy(gw_hbm, gw, sems.at[SEM_GW])
    cp_bx = pltpu.make_async_copy(bx_hbm, bx, sems.at[SEM_BX])
    cp_wg = pltpu.make_async_copy(wg_hbm, wg, sems.at[SEM_WG])
    cp_wu = pltpu.make_async_copy(wu_hbm, wu, sems.at[SEM_WU])
    cp_wd = pltpu.make_async_copy(wd_hbm, wd, sems.at[SEM_WD])

    with _scope("prologue"):
        cp_wq(0).start()
        cp_ax0.start()
        for p in range(1, NWC):
            cp_wq(p).start()
        cp_ax1.start()

        def start_rest():
            cp_axr.start()
            cp_gw.start()
            cp_wo.start()
            cp_wg.start()
            cp_wu.start()
            cp_wd.start()
            cp_bx.start()

        LATE = CFG.get('late', 1)
        if not LATE:
            start_rest()
        flag[0] = 0
        t0[:, 0:HALO // 2, :] = jnp.zeros((3 * NCB, HALO // 2, LANES), jnp.uint32)
        cp_ax0.wait()
        PG = CFG.get('pg', 1)

        def body(i, carry):
            for k in range(PG):
                cp_wq(i * PG + k).wait()
            x = ax[0:TM, :]
            for k in range(PG):
                p = i * PG + k
                res = jnp.dot(x, wq[p], preferred_element_type=jnp.float32)
                for b in range(BPC):
                    blk = res[:, b * LANES:(b + 1) * LANES]
                    _put(t0, p * BPC + b, 0, blk)
                    _put(qkv, p * BPC + b, TM - HALO, blk[TM - HALO:, :])
            return carry

        lax.fori_loop(0, NWC // PG, body, 0)
        if LATE:
            start_rest()
        cp_ax1.wait()

    def phase_a(i, carry):
        @pl.when(i == 1)
        def _():
            cp_axr.wait()

        with _scope("phase_a"):
            r0 = pl.multiple_of(TM + i * TA, 16)
            for m in range((TM + HALO) // 16):
                _refill(t0, win, 0, m)
            x = ax[pl.ds(r0, TA), :]
            for p in range(NWC):
                res = jnp.dot(x, wq[p], preferred_element_type=jnp.float32)
                for b in range(BPC):
                    _put(qkv, p * BPC + b, r0, res[:, b * LANES:(b + 1) * LANES])
        return carry

    lax.fori_loop(0, NA, phase_a, 0)

    cp_gw.wait()
    cp_wo.wait()
    cp_wg.wait()
    cp_wu.wait()
    cp_wd.wait()
    cp_bx.wait()

    def phase_b(i, carry):
        @pl.when(i >= 2)
        def _():
            for g in range(OG):
                cp_out(i - 2, g).wait()

        with _scope("phase_b"):
            r0 = pl.multiple_of(i * TM, TM)
            never = flag[0] != 0
            nrg = TM // 8
            nblk = F // LANES

            def attn(rg):
                outs = _attention_rows(win, rg, r0)
                for j in range(NCB):
                    osc[8 * rg:8 * rg + 8, j * LANES:(j + 1) * LANES] = outs[j].astype(jnp.bfloat16)
                return outs[NCB - 1]

            x = bx[pl.ds(r0, TM), :]
            acc = None
            bpc = FC // LANES
            nslots = 2 * nblk
            s_first = CFG.get('s_first', 3)
            s_last = CFG.get('s_last', 50)
            rn = pl.multiple_of(jnp.minimum(i + 1, NT_ - 1) * TM, TM)

            def refill(m):
                return _refill(qkv, win, rn, m)

            attn_slot = [s_first + rg * (s_last - s_first + 1) // nrg for rg in range(nrg)]
            rdelay = CFG.get('rdelay', 2)
            npiece = (TM + HALO) // 16
            jobs = {}
            late = []
            for rg in range(nrg):
                jobs.setdefault(attn_slot[rg], []).append(functools.partial(attn, rg))
            for m in range(npiece):
                last_reader = min(2 * m + 1, nrg - 1)
                slot = attn_slot[last_reader] + rdelay
                if slot < nslots:
                    jobs.setdefault(slot, []).append(functools.partial(refill, m))
                else:
                    late.append(m)

            def lhs(slot):
                todo = jobs.get(slot, [])
                if not todo:
                    return x
                tiles = []
                for k, job in enumerate(todo):
                    dep = job()
                    depb = jnp.concatenate([dep, dep], axis=0).astype(jnp.bfloat16)
                    tiles.append(jnp.where(never, depb, x[0:16, k * LANES:(k + 1) * LANES]))
                top = jnp.concatenate(tiles + [x[0:16, len(todo) * LANES:]], axis=1)
                return jnp.concatenate([top, x[16:, :]], axis=0)

            for c in range(F // FC):
                hs = []
                for b in range(bpc):
                    n = c * bpc + b
                    cols = slice(n * LANES, (n + 1) * LANES)
                    g = jnp.dot(lhs(2 * n), wg[:, cols], preferred_element_type=jnp.float32)
                    u = jnp.dot(lhs(2 * n + 1), wu[:, cols], preferred_element_type=jnp.float32)
                    hs.append((jax.nn.gelu(g, approximate=True) * u).astype(jnp.bfloat16))
                h = jnp.concatenate(hs, axis=1)
                d = jnp.dot(h, wd[c * FC:(c + 1) * FC, :], preferred_element_type=jnp.float32)
                acc = d if acc is None else acc + d

            for m in late:
                refill(m)

            gate = _gate(ax[pl.ds(r0, TM), :], gw)
            a = jnp.dot(osc[...], wo[...], preferred_element_type=jnp.float32)
            slot = i % 2
            for cb in range(NCB):
                cols = slice(cb * LANES, (cb + 1) * LANES)
                obuf[slot, :, cols] = (gate * a[:, cols] + (1.0 - gate) * acc[:, cols]).astype(jnp.bfloat16)
                if ((cb + 1) * LANES) % OW == 0 and (cb + 1) * LANES < D:
                    cp_out(i, (cb + 1) * LANES // OW - 1).start()
        cp_out(i, OG - 1).start()
        return carry

    lax.fori_loop(0, NT_, phase_b, 0)
    for g in range(OG):
        cp_out(NT_ - 2, g).wait()
    for g in range(OG):
        cp_out(NT_ - 1, g).wait()


@jax.jit
def pallas_gated_mix__sliding_local_dilated__glu_gated_geglu__prompt_kernel(
    A_x, A_wqkv, A_wo, B_x, B_w_gate, B_w_up, B_w_down, gate_w,
):
    bf16 = jnp.bfloat16
    any_spec = pl.BlockSpec(memory_space=pl.ANY)
    out = pl.pallas_call(
        _kernel,
        in_specs=[any_spec] * 8,
        out_specs=any_spec,
        out_shape=jax.ShapeDtypeStruct((S, D), bf16),
        scratch_shapes=[
            pltpu.VMEM((S, D), bf16),
            pltpu.VMEM((S, D), bf16),
            pltpu.VMEM((NWC, D, WC), bf16),
            pltpu.VMEM((D, D), bf16),
            pltpu.VMEM((D, F), bf16),
            pltpu.VMEM((D, F), bf16),
            pltpu.VMEM((F, D), bf16),
            pltpu.VMEM((D,), bf16),
            pltpu.VMEM((3 * NCB, (HALO + S) // 2 + CFG.get('padq', 0), LANES), jnp.uint32),
            pltpu.VMEM((3 * NCB, (HALO + TM) // 2, LANES), jnp.uint32),
            pltpu.VMEM((3 * NCB, HALO + TM + CFG.get('padw', 0), LANES), jnp.float32),
            pltpu.VMEM((TM, D), bf16),
            pltpu.VMEM((2, TM, D), bf16),
            pltpu.SMEM((1,), jnp.int32),
            pltpu.SemaphoreType.DMA((NSEM,)),
        ],
        compiler_params=pltpu.CompilerParams(
            vmem_limit_bytes=120 * 1024 * 1024,
            disable_bounds_checks=bool(CFG.get('nochk', 1)),
            disable_semaphore_checks=bool(CFG.get('nochk', 1)),
        ),
    )(A_x.reshape(S, D), A_wqkv, A_wo, B_x.reshape(S, D), B_w_gate, B_w_up,
      B_w_down, gate_w)
    return out.reshape(1, S, D)
```

```python
import functools

import jax
import jax.numpy as jnp
from jax import lax
from jax.experimental import pallas as pl
from jax.experimental.pallas import tpu as pltpu

S = 2048
D = 1024
F = 3584
DH = 32
W = 8
DIL = 2
HALO = 16
LANES = 128
NCB = D // LANES

TM = 256
NT = S // TM
TA = 448
NA = (S - TM) // TA
assert TM + NA * TA == S
FC = 256
WC = 256
NWC = 3 * D // WC
BPC = WC // LANES
NPIECE = (TM + HALO) // 16
WIN_ROWS = HALO + TM + 8

SLOT_FIRST = 3
SLOT_LAST = 54
REFILL_DELAY = 1

(SEM_AX0, SEM_AX1, SEM_AXR, SEM_GW, SEM_BX, SEM_WG, SEM_WU, SEM_WD, SEM_WO) = range(9)
SEM_WQ = 9
SEM_OUT = SEM_WQ + NWC
NSEM = SEM_OUT + 2 * NCB

QSCALE = DH ** -0.5


def _head_align(blocks):
    rows = list(blocks)
    lane = lax.broadcasted_iota(jnp.int32, rows[0].shape, 1)
    for s in range(3):
        shift = 4 << s
        low = (lane & shift) == 0
        for b in range(NCB):
            if b & (1 << s):
                continue
            b2 = b | (1 << s)
            lo_row, hi_row = rows[b], rows[b2]
            rows[b] = jnp.where(low, lo_row, pltpu.roll(hi_row, shift, 1))
            rows[b2] = jnp.where(low, pltpu.roll(lo_row, LANES - shift, 1), hi_row)
    return rows


def _attention_rows(win, rg, row0):
    base = HALO + 8 * rg
    q = [win[j, base:base + 8, :] for j in range(NCB)]
    lane = lax.broadcasted_iota(jnp.int32, (8, LANES), 1)
    logits = []
    for w in range(W):
        lo = base - DIL * w
        s = None
        for j in range(NCB):
            t = q[j] * win[NCB + j, lo:lo + 8, :]
            s = t if s is None else s + t
        s = s + pltpu.roll(s, 1, 1)
        s = s + pltpu.roll(s, 2, 1)
        if 8 * rg < DIL * w:
            row = row0 + 8 * rg + lax.broadcasted_iota(jnp.int32, (8, LANES), 0)
            s = jnp.where(row >= DIL * w, s, -1e9)
        logits.append(s)
    m = logits[0]
    for w in range(1, W):
        m = jnp.maximum(m, logits[w])
    p = [jnp.exp(s - m) for s in logits]
    den = p[0]
    for w in range(1, W):
        den = den + p[w]
    inv = 1.0 / den
    p = [pw * inv for pw in p]
    outs = []
    for j in range(NCB):
        idx = (lane // DH) * DH + (4 * j + 3)
        o = None
        for w in range(W):
            lo = base - DIL * w
            t = jnp.take_along_axis(p[w], idx, axis=1) * win[2 * NCB + j, lo:lo + 8, :]
            o = t if o is None else o + t
        outs.append(o)
    return outs


def _pack(blk):
    return pltpu.bitcast(blk.astype(jnp.bfloat16), jnp.uint32)


def _unpack(words):
    return pltpu.bitcast(words, jnp.bfloat16).astype(jnp.float32)


def _put(buf, jj, r0, blk):
    start = (r0 + HALO) // 2
    if not isinstance(r0, int):
        start = pl.multiple_of(start, 8)
    buf[jj, pl.ds(start, blk.shape[0] // 2), :] = _pack(blk)


def _aligned_rows(t0, start):
    vals = [_unpack(t0[jj, pl.ds(start, 8), :]) for jj in range(3 * NCB)]
    return ([blk * QSCALE for blk in _head_align(vals[0:NCB])]
            + _head_align(vals[NCB:2 * NCB]) + vals[2 * NCB:])


def _refill(qkv, win, row0, m):
    start = pl.multiple_of(row0 // 2 + 8 * m, 8)
    val = None
    for jj in range(3 * NCB):
        val = _unpack(qkv[jj, pl.ds(start, 8), :])
        win[jj, 16 * m:16 * m + 16, :] = val
    return val[0:8, :]


def _kernel(ax_hbm, wqkv_hbm, wo_hbm, bx_hbm, wg_hbm, wu_hbm, wd_hbm, gw_hbm,
            out_hbm,
            ax, bx, wq, wo, wg, wu, wd, gw, qkv, t0, win, osc, obuf, flag, sems):

    def copy(src, dst, sem):
        return pltpu.make_async_copy(src, dst, sems.at[sem])

    def cp_wq(p):
        return copy(wqkv_hbm.at[:, pl.ds(p * WC, WC)], wq.at[p], SEM_WQ + p)

    def cp_ax(start, size, sem):
        return copy(ax_hbm.at[pl.ds(start, size), :], ax.at[pl.ds(start, size), :], sem)

    def cp_out(i, g):
        slot = i % 2
        return copy(obuf.at[slot, :, pl.ds(g * LANES, LANES)],
                    out_hbm.at[pl.ds(pl.multiple_of(i * TM, TM), TM), pl.ds(g * LANES, LANES)],
                    SEM_OUT + slot * NCB + g)

    cp_ax0 = cp_ax(0, TM, SEM_AX0)
    cp_ax1 = cp_ax(TM, TA, SEM_AX1)
    cp_axr = cp_ax(TM + TA, S - TM - TA, SEM_AXR)
    late_copies = [copy(gw_hbm, gw, SEM_GW), copy(wo_hbm, wo, SEM_WO), copy(wg_hbm, wg, SEM_WG),
                   copy(wu_hbm, wu, SEM_WU), copy(wd_hbm, wd, SEM_WD), copy(bx_hbm, bx, SEM_BX)]

    cp_wq(0).start()
    cp_ax0.start()
    for p in range(1, NWC):
        cp_wq(p).start()
    cp_ax1.start()
    flag[0] = 0
    t0[:, 0:HALO // 2, :] = jnp.zeros((3 * NCB, HALO // 2, LANES), jnp.uint32)
    cp_ax0.wait()

    def first_tile(p, carry):
        cp_wq(p).wait()
        res = jnp.dot(ax[0:TM, :], wq[p], preferred_element_type=jnp.float32)
        for b in range(BPC):
            _put(t0, p * BPC + b, 0, res[:, b * LANES:(b + 1) * LANES])
        return carry

    lax.fori_loop(0, NWC, first_tile, 0)
    cp_axr.start()
    for cp in late_copies:
        cp.start()
    cp_ax1.wait()

    def phase_a(i, carry):
        @pl.when(i == 1)
        def _():
            cp_axr.wait()

        r0 = pl.multiple_of(TM + i * TA, 16)
        per_step = -(-NPIECE // NA)
        for k in range(per_step):
            m = jnp.minimum(i * per_step + k, NPIECE - 1)
            blocks = _aligned_rows(t0, pl.multiple_of(8 * m, 8))
            for jj in range(3 * NCB):
                win[jj, pl.ds(pl.multiple_of(16 * m, 16), 16), :] = blocks[jj]
        blocks = _aligned_rows(t0, TM // 2)
        for jj in range(3 * NCB):
            _put(qkv, jj, TM - HALO, blocks[jj])

        x = ax[pl.ds(r0, TA), :]
        blocks = []
        for p in range(NWC):
            res = jnp.dot(x, wq[p], preferred_element_type=jnp.float32)
            blocks += [res[:, b * LANES:(b + 1) * LANES] for b in range(BPC)]
            if p * BPC >= 2 * NCB:
                for jj in range(p * BPC, (p + 1) * BPC):
                    _put(qkv, jj, r0, blocks[jj])
        qa = _head_align(blocks[0:NCB])
        ka = _head_align(blocks[NCB:2 * NCB])
        for j in range(NCB):
            _put(qkv, j, r0, qa[j] * QSCALE)
            _put(qkv, NCB + j, r0, ka[j])
        return carry

    lax.fori_loop(0, NA, phase_a, 0)
    for cp in late_copies:
        cp.wait()

    def phase_b(i, carry):
        @pl.when(i >= 2)
        def _():
            for g in range(NCB):
                cp_out(i - 2, g).wait()

        r0 = pl.multiple_of(i * TM, TM)
        r_next = pl.multiple_of(jnp.minimum(i + 1, NT - 1) * TM, TM)
        never = flag[0] != 0
        nrg = TM // 8
        nslot = 2 * F // LANES

        def attend(rg):
            outs = _attention_rows(win, rg, r0)
            for j in range(NCB):
                osc[8 * rg:8 * rg + 8, j * LANES:(j + 1) * LANES] = outs[j].astype(jnp.bfloat16)
            return outs[NCB - 1]

        attend_slot = [SLOT_FIRST + rg * (SLOT_LAST - SLOT_FIRST + 1) // nrg for rg in range(nrg)]
        jobs = {}
        for rg in range(nrg):
            jobs.setdefault(attend_slot[rg], []).append(functools.partial(attend, rg))
        for m in range(NPIECE):
            slot = attend_slot[min(2 * m + 1, nrg - 1)] + REFILL_DELAY
            assert slot < nslot
            jobs.setdefault(slot, []).append(functools.partial(_refill, qkv, win, r_next, m))

        x = bx[pl.ds(r0, TM), :]

        def lhs(slot):
            todo = jobs.get(slot, [])
            if not todo:
                return x
            tiles = []
            for k, job in enumerate(todo):
                dep = job()
                dep = jnp.concatenate([dep, dep], axis=0).astype(jnp.bfloat16)
                tiles.append(jnp.where(never, dep, x[0:16, k * LANES:(k + 1) * LANES]))
            top = jnp.concatenate(tiles + [x[0:16, len(todo) * LANES:]], axis=1)
            return jnp.concatenate([top, x[16:, :]], axis=0)

        ffn = None
        for c in range(F // FC):
            hs = []
            for n in range(c * FC // LANES, (c + 1) * FC // LANES):
                cols = slice(n * LANES, (n + 1) * LANES)
                g = jnp.dot(lhs(2 * n), wg[:, cols], preferred_element_type=jnp.float32)
                u = jnp.dot(lhs(2 * n + 1), wu[:, cols], preferred_element_type=jnp.float32)
                hs.append((jax.nn.gelu(g, approximate=True) * u).astype(jnp.bfloat16))
            d = jnp.dot(jnp.concatenate(hs, axis=1), wd[c * FC:(c + 1) * FC, :],
                        preferred_element_type=jnp.float32)
            ffn = d if ffn is None else ffn + d

        xa = ax[pl.ds(r0, TM), :].astype(jnp.float32)
        gate_w = gw[...].astype(jnp.float32).reshape(1, D)
        gate = jax.nn.sigmoid(jnp.sum(xa * gate_w, axis=-1, keepdims=True))
        a = jnp.dot(osc[...], wo[...], preferred_element_type=jnp.float32)
        slot = i % 2
        for g in range(NCB):
            cols = slice(g * LANES, (g + 1) * LANES)
            obuf[slot, :, cols] = (gate * a[:, cols] + (1.0 - gate) * ffn[:, cols]).astype(jnp.bfloat16)
            cp_out(i, g).start()
        return carry

    lax.fori_loop(0, NT, phase_b, 0)
    for i in (NT - 2, NT - 1):
        for g in range(NCB):
            cp_out(i, g).wait()


@jax.jit
def pallas_gated_mix__sliding_local_dilated__glu_gated_geglu__prompt_kernel(
    A_x: jax.Array,
    A_wqkv: jax.Array,
    A_wo: jax.Array,
    B_x: jax.Array,
    B_w_gate: jax.Array,
    B_w_up: jax.Array,
    B_w_down: jax.Array,
    gate_w: jax.Array,
):
    bf16 = jnp.bfloat16
    hbm = pl.BlockSpec(memory_space=pl.ANY)
    out = pl.pallas_call(
        _kernel,
        in_specs=[hbm] * 8,
        out_specs=hbm,
        out_shape=jax.ShapeDtypeStruct((S, D), bf16),
        scratch_shapes=[
            pltpu.VMEM((S, D), bf16),
            pltpu.VMEM((S, D), bf16),
            pltpu.VMEM((NWC, D, WC), bf16),
            pltpu.VMEM((D, D), bf16),
            pltpu.VMEM((D, F), bf16),
            pltpu.VMEM((D, F), bf16),
            pltpu.VMEM((F, D), bf16),
            pltpu.VMEM((D,), bf16),
            pltpu.VMEM((3 * NCB, (HALO + S) // 2, LANES), jnp.uint32),
            pltpu.VMEM((3 * NCB, (HALO + TM) // 2, LANES), jnp.uint32),
            pltpu.VMEM((3 * NCB, WIN_ROWS, LANES), jnp.float32),
            pltpu.VMEM((TM, D), bf16),
            pltpu.VMEM((2, TM, D), bf16),
            pltpu.SMEM((1,), jnp.int32),
            pltpu.SemaphoreType.DMA((NSEM,)),
        ],
        compiler_params=pltpu.CompilerParams(
            vmem_limit_bytes=120 * 1024 * 1024,
            disable_bounds_checks=True,
            disable_semaphore_checks=True,
        ),
    )(A_x.reshape(S, D), A_wqkv, A_wo, B_x.reshape(S, D), B_w_gate, B_w_up, B_w_down, gate_w)
    return out.reshape(1, S, D)
```

```python
import functools

import jax
import jax.numpy as jnp
from jax import lax
from jax.experimental import pallas as pl
from jax.experimental.pallas import tpu as pltpu

S = 2048
D = 1024
F = 3584
DH = 32
W = 8
DIL = 2
HALO = 16
LANES = 128
NCB = D // LANES

TM = 256
NT = S // TM
TA = 448
NA = (S - TM) // TA
assert TM + NA * TA == S
FC = 256
WC = 256
NWC = 3 * D // WC
BPC = WC // LANES
NPIECE = (TM + HALO) // 16
WIN_ROWS = HALO + TM + 8

SLOT_FIRST = 3
SLOT_LAST = 53

(SEM_AX0, SEM_AX1, SEM_AXR, SEM_GW, SEM_BX, SEM_WG, SEM_WU, SEM_WD, SEM_WO) = range(9)
SEM_WQ = 9
SEM_OUT = SEM_WQ + NWC
NSEM = SEM_OUT + 2 * NCB

QSCALE = DH ** -0.5


def _head_align(blocks):
    rows = list(blocks)
    lane = lax.broadcasted_iota(jnp.int32, rows[0].shape, 1)
    for s in range(3):
        shift = 4 << s
        low = (lane & shift) == 0
        for b in range(NCB):
            if b & (1 << s):
                continue
            b2 = b | (1 << s)
            lo_row, hi_row = rows[b], rows[b2]
            rows[b] = jnp.where(low, lo_row, pltpu.roll(hi_row, shift, 1))
            rows[b2] = jnp.where(low, pltpu.roll(lo_row, LANES - shift, 1), hi_row)
    return rows


def _attention_rows(win, rg, row0):
    base = HALO + 8 * rg
    q = [win[j, base:base + 8, :] for j in range(NCB)]
    lane = lax.broadcasted_iota(jnp.int32, (8, LANES), 1)
    logits = []
    for w in range(W):
        lo = base - DIL * w
        s = None
        for j in range(NCB):
            t = q[j] * win[NCB + j, lo:lo + 8, :]
            s = t if s is None else s + t
        s = s + pltpu.roll(s, 1, 1)
        s = s + pltpu.roll(s, 2, 1)
        if 8 * rg < DIL * w:
            row = row0 + 8 * rg + lax.broadcasted_iota(jnp.int32, (8, LANES), 0)
            s = jnp.where(row >= DIL * w, s, -1e9)
        logits.append(s)
    m = logits[0]
    for w in range(1, W):
        m = jnp.maximum(m, logits[w])
    p = [jnp.exp(s - m) for s in logits]
    den = p[0]
    for w in range(1, W):
        den = den + p[w]
    inv = 1.0 / den
    p = [pw * inv for pw in p]
    outs = []
    for j in range(NCB):
        idx = (lane // DH) * DH + (4 * j + 3)
        o = None
        for w in range(W):
            lo = base - DIL * w
            t = jnp.take_along_axis(p[w], idx, axis=1) * win[2 * NCB + j, lo:lo + 8, :]
            o = t if o is None else o + t
        outs.append(o)
    return outs


def _put(buf, jj, r0, blk):
    start = r0 + HALO
    if not isinstance(r0, int):
        start = pl.multiple_of(start, 16)
    buf[jj, pl.ds(start, blk.shape[0]), :] = blk.astype(jnp.bfloat16)


def _get16(buf, jj, start):
    return buf[jj, pl.ds(start, 16), :].astype(jnp.float32)


def _aligned_rows(t0, start):
    vals = [_get16(t0, jj, start) for jj in range(3 * NCB)]
    return ([blk * QSCALE for blk in _head_align(vals[0:NCB])]
            + _head_align(vals[NCB:2 * NCB]) + vals[2 * NCB:])


def _refill(qkv, win, row0, m):
    start = pl.multiple_of(row0 + 16 * m, 16)
    val = None
    for jj in range(3 * NCB):
        val = _get16(qkv, jj, start)
        win[jj, 16 * m:16 * m + 16, :] = val
    return val[0:8, :]


def _kernel(ax_hbm, wqkv_hbm, wo_hbm, bx_hbm, wg_hbm, wu_hbm, wd_hbm, gw_hbm,
            out_hbm,
            ax, bx, wq, wo, wg, wu, wd, gw, qkv, t0, win, osc, obuf, flag, sems):

    def copy(src, dst, sem):
        return pltpu.make_async_copy(src, dst, sems.at[sem])

    def cp_wq(p):
        return copy(wqkv_hbm.at[:, pl.ds(p * WC, WC)], wq.at[p], SEM_WQ + p)

    def cp_ax(start, size, sem):
        return copy(ax_hbm.at[pl.ds(start, size), :], ax.at[pl.ds(start, size), :], sem)

    def cp_out(i, g):
        slot = i % 2
        return copy(obuf.at[slot, :, pl.ds(g * LANES, LANES)],
                    out_hbm.at[pl.ds(pl.multiple_of(i * TM, TM), TM), pl.ds(g * LANES, LANES)],
                    SEM_OUT + slot * NCB + g)

    cp_ax0 = cp_ax(0, TM, SEM_AX0)
    cp_ax1 = cp_ax(TM, TA, SEM_AX1)
    cp_axr = cp_ax(TM + TA, S - TM - TA, SEM_AXR)
    late_copies = [copy(gw_hbm, gw, SEM_GW), copy(wo_hbm, wo, SEM_WO), copy(wg_hbm, wg, SEM_WG),
                   copy(wu_hbm, wu, SEM_WU), copy(wd_hbm, wd, SEM_WD), copy(bx_hbm, bx, SEM_BX)]

    cp_wq(0).start()
    cp_ax0.start()
    for p in range(1, NWC):
        cp_wq(p).start()
    cp_ax1.start()
    flag[0] = 0
    t0[:, 0:HALO, :] = jnp.zeros((3 * NCB, HALO, LANES), jnp.bfloat16)
    cp_ax0.wait()

    def first_tile(p, carry):
        cp_wq(p).wait()
        res = jnp.dot(ax[0:TM, :], wq[p], preferred_element_type=jnp.float32)
        for b in range(BPC):
            _put(t0, p * BPC + b, 0, res[:, b * LANES:(b + 1) * LANES])
        return carry

    lax.fori_loop(0, NWC, first_tile, 0)
    cp_axr.start()
    for cp in late_copies:
        cp.start()
    cp_ax1.wait()

    def phase_a(i, carry):
        @pl.when(i == 1)
        def _():
            cp_axr.wait()

        r0 = pl.multiple_of(TM + i * TA, 16)
        per_step = -(-NPIECE // NA)
        for k in range(per_step):
            m = jnp.minimum(i * per_step + k, NPIECE - 1)
            blocks = _aligned_rows(t0, pl.multiple_of(16 * m, 16))
            for jj in range(3 * NCB):
                win[jj, pl.ds(pl.multiple_of(16 * m, 16), 16), :] = blocks[jj]
        blocks = _aligned_rows(t0, TM)
        for jj in range(3 * NCB):
            _put(qkv, jj, TM - HALO, blocks[jj])

        x = ax[pl.ds(r0, TA), :]
        blocks = []
        for p in range(NWC):
            res = jnp.dot(x, wq[p], preferred_element_type=jnp.float32)
            blocks += [res[:, b * LANES:(b + 1) * LANES] for b in range(BPC)]
            if p * BPC >= 2 * NCB:
                for jj in range(p * BPC, (p + 1) * BPC):
                    _put(qkv, jj, r0, blocks[jj])
        qa = _head_align(blocks[0:NCB])
        ka = _head_align(blocks[NCB:2 * NCB])
        for j in range(NCB):
            _put(qkv, j, r0, qa[j] * QSCALE)
            _put(qkv, NCB + j, r0, ka[j])
        return carry

    lax.fori_loop(0, NA, phase_a, 0)
    for cp in late_copies:
        cp.wait()

    def phase_b(i, carry):
        @pl.when(i >= 2)
        def _():
            for g in range(NCB):
                cp_out(i - 2, g).wait()

        r0 = pl.multiple_of(i * TM, TM)
        r_next = pl.multiple_of(jnp.minimum(i + 1, NT - 1) * TM, TM)
        never = flag[0] != 0
        nrg = TM // 8
        nslot = 2 * F // LANES

        def attend(rg):
            outs = _attention_rows(win, rg, r0)
            for j in range(NCB):
                osc[8 * rg:8 * rg + 8, j * LANES:(j + 1) * LANES] = outs[j].astype(jnp.bfloat16)
            return outs[NCB - 1]

        seq = []
        for rg in range(nrg):
            seq.append(functools.partial(attend, rg))
            if rg % 2 == 1:
                seq.append(functools.partial(_refill, qkv, win, r_next, rg // 2))
        seq.append(functools.partial(_refill, qkv, win, r_next, NPIECE - 1))
        jobs = {}
        assert SLOT_LAST < nslot
        for k, job in enumerate(seq):
            jobs.setdefault(SLOT_FIRST + k * (SLOT_LAST - SLOT_FIRST + 1) // len(seq), []).append(job)

        x = bx[pl.ds(r0, TM), :]

        def lhs(slot):
            todo = jobs.get(slot, [])
            if not todo:
                return x
            tiles = []
            for k, job in enumerate(todo):
                dep = job()
                dep = jnp.concatenate([dep, dep], axis=0).astype(jnp.bfloat16)
                tiles.append(jnp.where(never, dep, x[0:16, k * LANES:(k + 1) * LANES]))
            top = jnp.concatenate(tiles + [x[0:16, len(todo) * LANES:]], axis=1)
            return jnp.concatenate([top, x[16:, :]], axis=0)

        ffn = None
        for c in range(F // FC):
            hs = []
            for n in range(c * FC // LANES, (c + 1) * FC // LANES):
                cols = slice(n * LANES, (n + 1) * LANES)
                g = jnp.dot(lhs(2 * n), wg[:, cols], preferred_element_type=jnp.float32)
                u = jnp.dot(lhs(2 * n + 1), wu[:, cols], preferred_element_type=jnp.float32)
                hs.append((jax.nn.gelu(g, approximate=True) * u).astype(jnp.bfloat16))
            d = jnp.dot(jnp.concatenate(hs, axis=1), wd[c * FC:(c + 1) * FC, :],
                        preferred_element_type=jnp.float32)
            ffn = d if ffn is None else ffn + d

        xa = ax[pl.ds(r0, TM), :].astype(jnp.float32)
        gate_w = gw[...].astype(jnp.float32).reshape(1, D)
        gate = jax.nn.sigmoid(jnp.sum(xa * gate_w, axis=-1, keepdims=True))
        a = jnp.dot(osc[...], wo[...], preferred_element_type=jnp.float32)
        slot = i % 2
        for g in range(NCB):
            cols = slice(g * LANES, (g + 1) * LANES)
            obuf[slot, :, cols] = (gate * a[:, cols] + (1.0 - gate) * ffn[:, cols]).astype(jnp.bfloat16)
            cp_out(i, g).start()
        return carry

    lax.fori_loop(0, NT, phase_b, 0)
    for i in (NT - 2, NT - 1):
        for g in range(NCB):
            cp_out(i, g).wait()


@jax.jit
def pallas_gated_mix__sliding_local_dilated__glu_gated_geglu__prompt_kernel(
    A_x: jax.Array,
    A_wqkv: jax.Array,
    A_wo: jax.Array,
    B_x: jax.Array,
    B_w_gate: jax.Array,
    B_w_up: jax.Array,
    B_w_down: jax.Array,
    gate_w: jax.Array,
):
    bf16 = jnp.bfloat16
    hbm = pl.BlockSpec(memory_space=pl.ANY)
    out = pl.pallas_call(
        _kernel,
        in_specs=[hbm] * 8,
        out_specs=hbm,
        out_shape=jax.ShapeDtypeStruct((S, D), bf16),
        scratch_shapes=[
            pltpu.VMEM((S, D), bf16),
            pltpu.VMEM((S, D), bf16),
            pltpu.VMEM((NWC, D, WC), bf16),
            pltpu.VMEM((D, D), bf16),
            pltpu.VMEM((D, F), bf16),
            pltpu.VMEM((D, F), bf16),
            pltpu.VMEM((F, D), bf16),
            pltpu.VMEM((D,), bf16),
            pltpu.VMEM((3 * NCB, HALO + S, LANES), bf16),
            pltpu.VMEM((3 * NCB, HALO + TM, LANES), bf16),
            pltpu.VMEM((3 * NCB, WIN_ROWS, LANES), jnp.float32),
            pltpu.VMEM((TM, D), bf16),
            pltpu.VMEM((2, TM, D), bf16),
            pltpu.SMEM((1,), jnp.int32),
            pltpu.SemaphoreType.DMA((NSEM,)),
        ],
        compiler_params=pltpu.CompilerParams(
            vmem_limit_bytes=120 * 1024 * 1024,
            disable_bounds_checks=True,
            disable_semaphore_checks=True,
        ),
    )(A_x.reshape(S, D), A_wqkv, A_wo, B_x.reshape(S, D), B_w_gate, B_w_up, B_w_down, gate_w)
    return out.reshape(1, S, D)
```

```python
import functools

import jax
import jax.numpy as jnp
from jax import lax
from jax.experimental import pallas as pl
from jax.experimental.pallas import tpu as pltpu

S = 2048
D = 1024
F = 3584
DH = 32
W = 8
DIL = 2
HALO = 16
LANES = 128
NCB = D // LANES

TM = 256
NT = S // TM
TA = 448
NA = (S - TM) // TA
assert TM + NA * TA == S and NA >= 3
FC = 256
WC = 256
NWC = 3 * D // WC
BPC = WC // LANES
NPIECE = (TM + HALO) // 16
WIN_ROWS = HALO + TM + 8

SLOT_FIRST = 3
SLOT_LAST = 53
SPLIT = (0, NPIECE - 1, NPIECE)

(SEM_AX0, SEM_AX1, SEM_AXR, SEM_GW, SEM_BX0, SEM_BXR, SEM_WG, SEM_WU, SEM_WD, SEM_WO) = range(10)
SEM_STG = 10
SEM_AST = SEM_STG + 2
SEM_WQ = SEM_AST + 2
SEM_OUT = SEM_WQ + NWC
NSEM = SEM_OUT + 2 * NCB

QSCALE = DH ** -0.5


def _head_align(blocks):
    rows = list(blocks)
    lane = lax.broadcasted_iota(jnp.int32, rows[0].shape, 1)
    for s in range(3):
        shift = 4 << s
        low = (lane & shift) == 0
        for b in range(NCB):
            if b & (1 << s):
                continue
            b2 = b | (1 << s)
            lo_row, hi_row = rows[b], rows[b2]
            rows[b] = jnp.where(low, lo_row, pltpu.roll(hi_row, shift, 1))
            rows[b2] = jnp.where(low, pltpu.roll(lo_row, LANES - shift, 1), hi_row)
    return rows


def _attention_rows(win, rg, row0):
    base = HALO + 8 * rg
    q = [win[j, base:base + 8, :] for j in range(NCB)]
    lane = lax.broadcasted_iota(jnp.int32, (8, LANES), 1)
    logits = []
    for w in range(W):
        lo = base - DIL * w
        s = None
        for j in range(NCB):
            t = q[j] * win[NCB + j, lo:lo + 8, :]
            s = t if s is None else s + t
        s = s + pltpu.roll(s, 1, 1)
        s = s + pltpu.roll(s, 2, 1)
        if 8 * rg < DIL * w:
            row = row0 + 8 * rg + lax.broadcasted_iota(jnp.int32, (8, LANES), 0)
            s = jnp.where(row >= DIL * w, s, -1e9)
        logits.append(s)
    m = logits[0]
    for w in range(1, W):
        m = jnp.maximum(m, logits[w])
    p = [jnp.exp(s - m) for s in logits]
    den = p[0]
    for w in range(1, W):
        den = den + p[w]
    inv = 1.0 / den
    p = [pw * inv for pw in p]
    outs = []
    for j in range(NCB):
        idx = (lane // DH) * DH + (4 * j + 3)
        o = None
        for w in range(W):
            lo = base - DIL * w
            t = jnp.take_along_axis(p[w], idx, axis=1) * win[2 * NCB + j, lo:lo + 8, :]
            o = t if o is None else o + t
        outs.append(o)
    return outs


def _aligned_rows(t0, start):
    vals = [t0[jj, pl.ds(start, 16), :].astype(jnp.float32) for jj in range(3 * NCB)]
    return ([blk * QSCALE for blk in _head_align(vals[0:NCB])]
            + _head_align(vals[NCB:2 * NCB]) + vals[2 * NCB:])


def _refill(stg, win, m):
    val = None
    for jj in range(3 * NCB):
        val = stg[jj, 16 * m:16 * m + 16, :].astype(jnp.float32)
        win[jj, 16 * m:16 * m + 16, :] = val
    return val[0:8, :]


def _kernel(ax_hbm, wqkv_hbm, wo_hbm, bx_hbm, wg_hbm, wu_hbm, wd_hbm, gw_hbm,
            out_hbm, kvh_hbm,
            ax, bx, wq, wo, wg, wu, wd, gw, ast, stg, t0, win, osc, obuf, flag, sems):

    def copy(src, dst, sem):
        return pltpu.make_async_copy(src, dst, sems.at[sem])

    def cp_rows(src, dst, start, size, sem):
        return copy(src.at[pl.ds(start, size), :], dst.at[pl.ds(start, size), :], sem)

    def cp_wq(p):
        return copy(wqkv_hbm.at[:, pl.ds(p * WC, WC)], wq.at[p], SEM_WQ + p)

    def cp_ast(i):
        return copy(ast.at[i % 2], kvh_hbm.at[:, pl.ds(pl.multiple_of(i * TA, 16), TA), :],
                    SEM_AST + i % 2)

    def cp_stg(t, part):
        lo, hi = 16 * SPLIT[part], 16 * SPLIT[part + 1]
        return copy(kvh_hbm.at[:, pl.ds(pl.multiple_of((t - 1) * TM - HALO + lo, 16), hi - lo), :],
                    stg.at[:, pl.ds(lo, hi - lo), :], SEM_STG + part)

    def cp_out(i, g):
        slot = i % 2
        return copy(obuf.at[slot, :, pl.ds(g * LANES, LANES)],
                    out_hbm.at[pl.ds(pl.multiple_of(i * TM, TM), TM), pl.ds(g * LANES, LANES)],
                    SEM_OUT + slot * NCB + g)

    cp_ax0 = cp_rows(ax_hbm, ax, 0, TM, SEM_AX0)
    cp_ax1 = cp_rows(ax_hbm, ax, TM, TA, SEM_AX1)
    cp_axr = cp_rows(ax_hbm, ax, TM + TA, S - TM - TA, SEM_AXR)
    cp_bxr = cp_rows(bx_hbm, bx, TM, S - TM, SEM_BXR)
    late_copies = [copy(gw_hbm, gw, SEM_GW), copy(wo_hbm, wo, SEM_WO), copy(wg_hbm, wg, SEM_WG),
                   copy(wu_hbm, wu, SEM_WU), copy(wd_hbm, wd, SEM_WD),
                   cp_rows(bx_hbm, bx, 0, TM, SEM_BX0)]
    cp_stg1 = copy(kvh_hbm.at[:, pl.ds(0, TM), :], stg.at[:, pl.ds(HALO, TM), :], SEM_STG)

    cp_wq(0).start()
    cp_ax0.start()
    for p in range(1, NWC):
        cp_wq(p).start()
    cp_ax1.start()
    flag[0] = 0
    t0[:, 0:HALO, :] = jnp.zeros((3 * NCB, HALO, LANES), jnp.bfloat16)
    cp_ax0.wait()

    def first_tile(p, carry):
        cp_wq(p).wait()
        res = jnp.dot(ax[0:TM, :], wq[p], preferred_element_type=jnp.float32)
        for b in range(BPC):
            t0[p * BPC + b, HALO:, :] = res[:, b * LANES:(b + 1) * LANES].astype(jnp.bfloat16)
        return carry

    lax.fori_loop(0, NWC, first_tile, 0)
    cp_axr.start()
    for cp in late_copies:
        cp.start()
    cp_ax1.wait()

    def phase_a(i, carry):
        @pl.when(i == 1)
        def _():
            cp_axr.wait()

        @pl.when(i >= 2)
        def _():
            cp_ast(i - 2).wait()

        @pl.when(i == 2)
        def _():
            cp_stg1.start()

        per_step = -(-NPIECE // NA)
        for k in range(per_step):
            start = pl.multiple_of(16 * jnp.minimum(i * per_step + k, NPIECE - 1), 16)
            blocks = _aligned_rows(t0, start)
            for jj in range(3 * NCB):
                win[jj, pl.ds(start, 16), :] = blocks[jj]
        blocks = _aligned_rows(t0, TM)
        for jj in range(3 * NCB):
            stg[jj, 0:HALO, :] = blocks[jj].astype(jnp.bfloat16)

        x = ax[pl.ds(pl.multiple_of(TM + i * TA, 16), TA), :]
        slot = i % 2
        blocks = []
        for p in range(NWC):
            res = jnp.dot(x, wq[p], preferred_element_type=jnp.float32)
            blocks += [res[:, b * LANES:(b + 1) * LANES] for b in range(BPC)]
            if p * BPC >= 2 * NCB:
                for jj in range(p * BPC, (p + 1) * BPC):
                    ast[slot, jj] = blocks[jj].astype(jnp.bfloat16)
        qa = _head_align(blocks[0:NCB])
        ka = _head_align(blocks[NCB:2 * NCB])
        for j in range(NCB):
            ast[slot, j] = (qa[j] * QSCALE).astype(jnp.bfloat16)
            ast[slot, NCB + j] = ka[j].astype(jnp.bfloat16)
        cp_ast(i).start()
        return carry

    lax.fori_loop(0, NA, phase_a, 0)
    for cp in late_copies:
        cp.wait()
    cp_bxr.start()

    def phase_b(i, carry):
        @pl.when(i >= 2)
        def _():
            for g in range(NCB):
                cp_out(i - 2, g).wait()

        @pl.when(i == 0)
        def _():
            cp_stg1.wait()

        @pl.when(i == 1)
        def _():
            cp_bxr.wait()
            cp_ast(NA - 2).wait()
            cp_ast(NA - 1).wait()

        @pl.when(i >= 1)
        def _():
            for part in range(len(SPLIT) - 1):
                cp_stg(jnp.minimum(i + 1, NT - 1), part).wait()

        r0 = pl.multiple_of(i * TM, TM)
        t_fetch = jnp.minimum(i + 2, NT - 1)
        never = flag[0] != 0
        nrg = TM // 8
        nslot = 2 * F // LANES

        def attend(rg):
            outs = _attention_rows(win, rg, r0)
            for j in range(NCB):
                osc[8 * rg:8 * rg + 8, j * LANES:(j + 1) * LANES] = outs[j].astype(jnp.bfloat16)
            return outs[NCB - 1]

        def refill(m):
            dep = _refill(stg, win, m)
            if m + 1 in SPLIT:
                cp_stg(t_fetch, SPLIT.index(m + 1) - 1).start()
            return dep

        seq = []
        for rg in range(nrg):
            seq.append(functools.partial(attend, rg))
            if rg % 2 == 1:
                seq.append(functools.partial(refill, rg // 2))
        seq.append(functools.partial(refill, NPIECE - 1))
        jobs = {}
        assert SLOT_LAST < nslot
        for k, job in enumerate(seq):
            jobs.setdefault(SLOT_FIRST + k * (SLOT_LAST - SLOT_FIRST + 1) // len(seq), []).append(job)

        x = bx[pl.ds(r0, TM), :]

        def lhs(slot):
            todo = jobs.get(slot, [])
            if not todo:
                return x
            tiles = []
            for k, job in enumerate(todo):
                dep = job()
                dep = jnp.concatenate([dep, dep], axis=0).astype(jnp.bfloat16)
                tiles.append(jnp.where(never, dep, x[0:16, k * LANES:(k + 1) * LANES]))
            top = jnp.concatenate(tiles + [x[0:16, len(todo) * LANES:]], axis=1)
            return jnp.concatenate([top, x[16:, :]], axis=0)

        ffn = None
        for c in range(F // FC):
            hs = []
            for n in range(c * FC // LANES, (c + 1) * FC // LANES):
                cols = slice(n * LANES, (n + 1) * LANES)
                g = jnp.dot(lhs(2 * n), wg[:, cols], preferred_element_type=jnp.float32)
                u = jnp.dot(lhs(2 * n + 1), wu[:, cols], preferred_element_type=jnp.float32)
                hs.append((jax.nn.gelu(g, approximate=True) * u).astype(jnp.bfloat16))
            d = jnp.dot(jnp.concatenate(hs, axis=1), wd[c * FC:(c + 1) * FC, :],
                        preferred_element_type=jnp.float32)
            ffn = d if ffn is None else ffn + d

        xa = ax[pl.ds(r0, TM), :].astype(jnp.float32)
        gate_w = gw[...].astype(jnp.float32).reshape(1, D)
        gate = jax.nn.sigmoid(jnp.sum(xa * gate_w, axis=-1, keepdims=True))
        a = jnp.dot(osc[...], wo[...], preferred_element_type=jnp.float32)
        slot = i % 2
        for g in range(NCB):
            cols = slice(g * LANES, (g + 1) * LANES)
            obuf[slot, :, cols] = (gate * a[:, cols] + (1.0 - gate) * ffn[:, cols]).astype(jnp.bfloat16)
            cp_out(i, g).start()
        return carry

    lax.fori_loop(0, NT, phase_b, 0)
    for part in range(len(SPLIT) - 1):
        cp_stg(NT - 1, part).wait()
    for i in (NT - 2, NT - 1):
        for g in range(NCB):
            cp_out(i, g).wait()


@jax.jit
def pallas_gated_mix__sliding_local_dilated__glu_gated_geglu__prompt_kernel(
    A_x: jax.Array,
    A_wqkv: jax.Array,
    A_wo: jax.Array,
    B_x: jax.Array,
    B_w_gate: jax.Array,
    B_w_up: jax.Array,
    B_w_down: jax.Array,
    gate_w: jax.Array,
):
    bf16 = jnp.bfloat16
    hbm = pl.BlockSpec(memory_space=pl.ANY)
    out, _ = pl.pallas_call(
        _kernel,
        in_specs=[hbm] * 8,
        out_specs=[hbm, hbm],
        out_shape=[jax.ShapeDtypeStruct((S, D), bf16),
                   jax.ShapeDtypeStruct((3 * NCB, S - TM, LANES), bf16)],
        scratch_shapes=[
            pltpu.VMEM((S, D), bf16),
            pltpu.VMEM((S, D), bf16),
            pltpu.VMEM((NWC, D, WC), bf16),
            pltpu.VMEM((D, D), bf16),
            pltpu.VMEM((D, F), bf16),
            pltpu.VMEM((D, F), bf16),
            pltpu.VMEM((F, D), bf16),
            pltpu.VMEM((D,), bf16),
            pltpu.VMEM((2, 3 * NCB, TA, LANES), bf16),
            pltpu.VMEM((3 * NCB, HALO + TM, LANES), bf16),
            pltpu.VMEM((3 * NCB, HALO + TM, LANES), bf16),
            pltpu.VMEM((3 * NCB, WIN_ROWS, LANES), jnp.float32),
            pltpu.VMEM((TM, D), bf16),
            pltpu.VMEM((2, TM, D), bf16),
            pltpu.SMEM((1,), jnp.int32),
            pltpu.SemaphoreType.DMA((NSEM,)),
        ],
        compiler_params=pltpu.CompilerParams(
            vmem_limit_bytes=120 * 1024 * 1024,
            disable_bounds_checks=True,
            disable_semaphore_checks=True,
        ),
    )(A_x.reshape(S, D), A_wqkv, A_wo, B_x.reshape(S, D), B_w_gate, B_w_up, B_w_down, gate_w)
    return out.reshape(1, S, D)
```

```python
import functools

import jax
import jax.numpy as jnp
from jax import lax
from jax.experimental import pallas as pl
from jax.experimental.pallas import tpu as pltpu

S = 2048
D = 1024
F = 3584
DH = 32
W = 8
DIL = 2
HALO = 16
LANES = 128
NCB = D // LANES

TM = 256
NT = S // TM
TA = 448
NA = (S - TM) // TA
assert TM + NA * TA == S and NA >= 3
FC = 256
WC = 256
NWC = 3 * D // WC
BPC = WC // LANES
NPIECE = (TM + HALO) // 16
WIN_ROWS = HALO + TM + 8

SLOT_FIRST = 3
SLOT_LAST = 53
SPLIT = (0, NPIECE - 1, NPIECE)

(SEM_AX0, SEM_AX1, SEM_AXR, SEM_GW, SEM_WG, SEM_WU, SEM_WD, SEM_WO) = range(8)
SEM_STG = 8
SEM_AST = SEM_STG + 2
SEM_WQ = SEM_AST + 2
SEM_OUT = SEM_WQ + NWC
NSEM = SEM_OUT + 2 * NCB

QSCALE = DH ** -0.5


def _head_align(blocks):
    rows = list(blocks)
    lane = lax.broadcasted_iota(jnp.int32, rows[0].shape, 1)
    for s in range(3):
        shift = 4 << s
        low = (lane & shift) == 0
        for b in range(NCB):
            if b & (1 << s):
                continue
            b2 = b | (1 << s)
            lo_row, hi_row = rows[b], rows[b2]
            rows[b] = jnp.where(low, lo_row, pltpu.roll(hi_row, shift, 1))
            rows[b2] = jnp.where(low, pltpu.roll(lo_row, LANES - shift, 1), hi_row)
    return rows


def _attention_rows(win, rg, row0):
    base = HALO + 8 * rg
    q = [win[j, base:base + 8, :] for j in range(NCB)]
    lane = lax.broadcasted_iota(jnp.int32, (8, LANES), 1)
    logits = []
    for w in range(W):
        lo = base - DIL * w
        s = None
        for j in range(NCB):
            t = q[j] * win[NCB + j, lo:lo + 8, :]
            s = t if s is None else s + t
        s = s + pltpu.roll(s, 1, 1)
        s = s + pltpu.roll(s, 2, 1)
        if 8 * rg < DIL * w:
            row = row0 + 8 * rg + lax.broadcasted_iota(jnp.int32, (8, LANES), 0)
            s = jnp.where(row >= DIL * w, s, -1e9)
        logits.append(s)
    m = logits[0]
    for w in range(1, W):
        m = jnp.maximum(m, logits[w])
    p = [jnp.exp(s - m) for s in logits]
    den = p[0]
    for w in range(1, W):
        den = den + p[w]
    inv = 1.0 / den
    p = [pw * inv for pw in p]
    outs = []
    for j in range(NCB):
        idx = (lane // DH) * DH + (4 * j + 3)
        o = None
        for w in range(W):
            lo = base - DIL * w
            t = jnp.take_along_axis(p[w], idx, axis=1) * win[2 * NCB + j, lo:lo + 8, :]
            o = t if o is None else o + t
        outs.append(o)
    return outs


def _aligned_rows(t0, start):
    vals = [t0[jj, pl.ds(start, 16), :].astype(jnp.float32) for jj in range(3 * NCB)]
    return ([blk * QSCALE for blk in _head_align(vals[0:NCB])]
            + _head_align(vals[NCB:2 * NCB]) + vals[2 * NCB:])


def _refill(stg, win, m):
    val = None
    for jj in range(3 * NCB):
        val = stg[jj, 16 * m:16 * m + 16, :].astype(jnp.float32)
        win[jj, 16 * m:16 * m + 16, :] = val
    return val[0:8, :]


def _kernel(ax_hbm, wqkv_hbm, wo_hbm, wg_hbm, wu_hbm, wd_hbm, gw_hbm,
            out_hbm, kvh_hbm,
            ax, wq, wo, wg, wu, wd, gw, ast, stg, t0, win, osc, obuf, flag, sems):

    def copy(src, dst, sem):
        return pltpu.make_async_copy(src, dst, sems.at[sem])

    def cp_ax(start, size, sem):
        return copy(ax_hbm.at[pl.ds(start, size), :], ax.at[pl.ds(start, size), :], sem)

    def cp_wq(p):
        return copy(wqkv_hbm.at[:, pl.ds(p * WC, WC)], wq.at[p], SEM_WQ + p)

    def cp_ast(i):
        return copy(ast.at[i % 2], kvh_hbm.at[:, pl.ds(pl.multiple_of(i * TA, 16), TA), :],
                    SEM_AST + i % 2)

    def cp_stg(t, part):
        lo, hi = 16 * SPLIT[part], 16 * SPLIT[part + 1]
        return copy(kvh_hbm.at[:, pl.ds(pl.multiple_of((t - 1) * TM - HALO + lo, 16), hi - lo), :],
                    stg.at[:, pl.ds(lo, hi - lo), :], SEM_STG + part)

    def cp_out(i, g):
        slot = i % 2
        return copy(obuf.at[slot, :, pl.ds(g * LANES, LANES)],
                    out_hbm.at[pl.ds(pl.multiple_of(i * TM, TM), TM), pl.ds(g * LANES, LANES)],
                    SEM_OUT + slot * NCB + g)

    cp_ax0 = cp_ax(0, TM, SEM_AX0)
    cp_ax1 = cp_ax(TM, TA, SEM_AX1)
    cp_axr = cp_ax(TM + TA, S - TM - TA, SEM_AXR)
    late_copies = [copy(gw_hbm, gw, SEM_GW), copy(wo_hbm, wo, SEM_WO), copy(wg_hbm, wg, SEM_WG),
                   copy(wu_hbm, wu, SEM_WU), copy(wd_hbm, wd, SEM_WD)]
    cp_stg1 = copy(kvh_hbm.at[:, pl.ds(0, TM), :], stg.at[:, pl.ds(HALO, TM), :], SEM_STG)

    cp_wq(0).start()
    cp_ax0.start()
    for p in range(1, NWC):
        cp_wq(p).start()
    cp_ax1.start()
    flag[0] = 0
    t0[:, 0:HALO, :] = jnp.zeros((3 * NCB, HALO, LANES), jnp.bfloat16)
    cp_ax0.wait()

    def first_tile(p, carry):
        cp_wq(p).wait()
        res = jnp.dot(ax[0:TM, :], wq[p], preferred_element_type=jnp.float32)
        for b in range(BPC):
            t0[p * BPC + b, HALO:, :] = res[:, b * LANES:(b + 1) * LANES].astype(jnp.bfloat16)
        return carry

    lax.fori_loop(0, NWC, first_tile, 0)
    cp_axr.start()
    for cp in late_copies:
        cp.start()
    cp_ax1.wait()

    def phase_a(i, carry):
        @pl.when(i == 1)
        def _():
            cp_axr.wait()

        @pl.when(i >= 2)
        def _():
            cp_ast(i - 2).wait()

        @pl.when(i == 2)
        def _():
            cp_stg1.start()

        per_step = -(-NPIECE // NA)
        for k in range(per_step):
            start = pl.multiple_of(16 * jnp.minimum(i * per_step + k, NPIECE - 1), 16)
            blocks = _aligned_rows(t0, start)
            for jj in range(3 * NCB):
                win[jj, pl.ds(start, 16), :] = blocks[jj]
        blocks = _aligned_rows(t0, TM)
        for jj in range(3 * NCB):
            stg[jj, 0:HALO, :] = blocks[jj].astype(jnp.bfloat16)

        x = ax[pl.ds(pl.multiple_of(TM + i * TA, 16), TA), :]
        slot = i % 2
        blocks = []
        for p in range(NWC):
            res = jnp.dot(x, wq[p], preferred_element_type=jnp.float32)
            blocks += [res[:, b * LANES:(b + 1) * LANES] for b in range(BPC)]
            if p * BPC >= 2 * NCB:
                for jj in range(p * BPC, (p + 1) * BPC):
                    ast[slot, jj] = blocks[jj].astype(jnp.bfloat16)
        qa = _head_align(blocks[0:NCB])
        ka = _head_align(blocks[NCB:2 * NCB])
        for j in range(NCB):
            ast[slot, j] = (qa[j] * QSCALE).astype(jnp.bfloat16)
            ast[slot, NCB + j] = ka[j].astype(jnp.bfloat16)
        cp_ast(i).start()
        return carry

    lax.fori_loop(0, NA, phase_a, 0)
    for cp in late_copies:
        cp.wait()

    def phase_b(i, carry):
        @pl.when(i >= 2)
        def _():
            for g in range(NCB):
                cp_out(i - 2, g).wait()

        @pl.when(i == 0)
        def _():
            cp_stg1.wait()

        @pl.when(i == 1)
        def _():
            cp_ast(NA - 2).wait()
            cp_ast(NA - 1).wait()

        @pl.when(jnp.logical_and(i >= 1, i + 1 < NT))
        def _():
            for part in range(len(SPLIT) - 1):
                cp_stg(i + 1, part).wait()

        r0 = pl.multiple_of(i * TM, TM)
        never = flag[0] != 0
        nrg = TM // 8
        nslot = 2 * F // LANES

        def attend(rg):
            outs = _attention_rows(win, rg, r0)
            for j in range(NCB):
                osc[8 * rg:8 * rg + 8, j * LANES:(j + 1) * LANES] = outs[j].astype(jnp.bfloat16)
            return outs[NCB - 1]

        def refill(m):
            dep = _refill(stg, win, m)
            if m + 1 in SPLIT:
                @pl.when(i + 2 < NT)
                def _():
                    cp_stg(i + 2, SPLIT.index(m + 1) - 1).start()
            return dep

        seq = []
        for rg in range(nrg):
            seq.append(functools.partial(attend, rg))
            if rg % 2 == 1:
                seq.append(functools.partial(refill, rg // 2))
        seq.append(functools.partial(refill, NPIECE - 1))
        jobs = {}
        assert SLOT_LAST < nslot
        for k, job in enumerate(seq):
            jobs.setdefault(SLOT_FIRST + k * (SLOT_LAST - SLOT_FIRST + 1) // len(seq), []).append(job)

        x = ax[pl.ds(r0, TM), :]

        def lhs(slot):
            todo = jobs.get(slot, [])
            if not todo:
                return x
            tiles = []
            for k, job in enumerate(todo):
                dep = job()
                dep = jnp.concatenate([dep, dep], axis=0).astype(jnp.bfloat16)
                tiles.append(jnp.where(never, dep, x[0:16, k * LANES:(k + 1) * LANES]))
            top = jnp.concatenate(tiles + [x[0:16, len(todo) * LANES:]], axis=1)
            return jnp.concatenate([top, x[16:, :]], axis=0)

        ffn = None
        for c in range(F // FC):
            hs = []
            for n in range(c * FC // LANES, (c + 1) * FC // LANES):
                cols = slice(n * LANES, (n + 1) * LANES)
                g = jnp.dot(lhs(2 * n), wg[:, cols], preferred_element_type=jnp.float32)
                u = jnp.dot(lhs(2 * n + 1), wu[:, cols], preferred_element_type=jnp.float32)
                hs.append((jax.nn.gelu(g, approximate=True) * u).astype(jnp.bfloat16))
            d = jnp.dot(jnp.concatenate(hs, axis=1), wd[c * FC:(c + 1) * FC, :],
                        preferred_element_type=jnp.float32)
            ffn = d if ffn is None else ffn + d

        gate_w = gw[...].astype(jnp.float32).reshape(1, D)
        gate = jax.nn.sigmoid(jnp.sum(x.astype(jnp.float32) * gate_w, axis=-1, keepdims=True))
        a = jnp.dot(osc[...], wo[...], preferred_element_type=jnp.float32)
        slot = i % 2
        for g in range(NCB):
            cols = slice(g * LANES, (g + 1) * LANES)
            obuf[slot, :, cols] = (gate * a[:, cols] + (1.0 - gate) * ffn[:, cols]).astype(jnp.bfloat16)
            cp_out(i, g).start()
        return carry

    lax.fori_loop(0, NT, phase_b, 0)
    for i in (NT - 2, NT - 1):
        for g in range(NCB):
            cp_out(i, g).wait()


@jax.jit
def pallas_gated_mix__sliding_local_dilated__glu_gated_geglu__prompt_kernel(
    A_x: jax.Array,
    A_wqkv: jax.Array,
    A_wo: jax.Array,
    B_x: jax.Array,
    B_w_gate: jax.Array,
    B_w_up: jax.Array,
    B_w_down: jax.Array,
    gate_w: jax.Array,
):
    bf16 = jnp.bfloat16
    hbm = pl.BlockSpec(memory_space=pl.ANY)
    out, _ = pl.pallas_call(
        _kernel,
        in_specs=[hbm] * 7,
        out_specs=[hbm, hbm],
        out_shape=[jax.ShapeDtypeStruct((S, D), bf16),
                   jax.ShapeDtypeStruct((3 * NCB, S - TM, LANES), bf16)],
        scratch_shapes=[
            pltpu.VMEM((S, D), bf16),
            pltpu.VMEM((NWC, D, WC), bf16),
            pltpu.VMEM((D, D), bf16),
            pltpu.VMEM((D, F), bf16),
            pltpu.VMEM((D, F), bf16),
            pltpu.VMEM((F, D), bf16),
            pltpu.VMEM((D,), bf16),
            pltpu.VMEM((2, 3 * NCB, TA, LANES), bf16),
            pltpu.VMEM((3 * NCB, HALO + TM, LANES), bf16),
            pltpu.VMEM((3 * NCB, HALO + TM, LANES), bf16),
            pltpu.VMEM((3 * NCB, WIN_ROWS, LANES), jnp.float32),
            pltpu.VMEM((TM, D), bf16),
            pltpu.VMEM((2, TM, D), bf16),
            pltpu.SMEM((1,), jnp.int32),
            pltpu.SemaphoreType.DMA((NSEM,)),
        ],
        compiler_params=pltpu.CompilerParams(
            vmem_limit_bytes=120 * 1024 * 1024,
            disable_bounds_checks=True,
            disable_semaphore_checks=True,
        ),
    )(A_x.reshape(S, D), A_wqkv, A_wo, B_w_gate, B_w_up, B_w_down, gate_w)
    return out.reshape(1, S, D)
```
